```python
import jax
import jax.numpy as jnp

def _softmax(x, axis=-1):
    return jax.nn.softmax(x, axis=axis)

def _gelu(x):
    return jax.nn.gelu(x, approximate=True)

def _silu(x):
    return jax.nn.silu(x)

def _sigmoid(x):
    return jax.nn.sigmoid(x)

def _layernorm(x, axis=-1, eps=1e-05):
    m = jnp.mean(x, axis=axis, keepdims=True)
    v = jnp.var(x, axis=axis, keepdims=True)
    return (x - m) / jnp.sqrt(v + eps)

def _scatter_add(tgt, idx, src, axis=0):
    return tgt.at[idx].add(src)

def _segment_sum(src, seg, n):
    return jax.ops.segment_sum(src, seg, n)

class _Rng:

    def __init__(self, key):
        self._k = key

    def _next(self):
        self._k, sub = jax.random.split(self._k)
        return sub

    def normal(self, shape):
        return jax.random.normal(self._next(), shape, dtype=jnp.bfloat16)

    def randint(self, lo, hi, shape):
        return jax.random.randint(self._next(), shape, lo, hi, dtype=jnp.int32)

    def uniform(self, shape, lo=0.0, hi=1.0):
        return jax.random.uniform(self._next(), shape, jnp.bfloat16, lo, hi)

    def permutation(self, n):
        return jax.random.permutation(self._next(), n)
kernel_name = 'recurrent_scan__memory_aug_recurrent_mem_tr__moe_arch_mod__prompt'

def setup_inputs():
    _rng = _Rng(jax.random.key(int.from_bytes(__import__("os").urandom(4), "little")))
    _w = lambda a: (lambda t: t.astype(jnp.bfloat16) if jnp.issubdtype(t.dtype, jnp.floating) else t)(jnp.asarray(a))

    def _A_setup():
        B, S, Dm = (1, 2048, 640)
        H, Dh = (32, 128)
        M, seg = (8, 32)
        seg = min(seg, S)
        S = S // seg * seg
        return {'x': _w((lambda *s: _rng.normal(s) * 0.05)(B, S, Dm)), 'mem0': _w((lambda *s: _rng.normal(s) * 0.05)(B, M, Dm)), 'Wq': _w((lambda *s: _rng.normal(s) * 0.05)(Dm, H, Dh) * Dm ** (-0.5)), 'Wk': _w((lambda *s: _rng.normal(s) * 0.05)(Dm, H, Dh) * Dm ** (-0.5)), 'Wv': _w((lambda *s: _rng.normal(s) * 0.05)(Dm, H, Dh) * Dm ** (-0.5)), 'Wo': _w((lambda *s: _rng.normal(s) * 0.05)(H, Dh, Dm) * (H * Dh) ** (-0.5)), 'seg_len': seg}
    _A_in = _A_setup()

    def _B_setup():
        B, S, D, F, C = (1, 2048, 640, 1728, 8)
        return {'x': _w((lambda *s: _rng.normal(s) * 0.05)(B, S, D)), 'w_r': _w((lambda *s: _rng.normal(s) * 0.05)(D)), 'w_gate': _w((lambda *s: _rng.normal(s) * 0.05)(D, F)), 'w_up': _w((lambda *s: _rng.normal(s) * 0.05)(D, F)), 'w_down': _w((lambda *s: _rng.normal(s) * 0.05)(F, D))}
    _B_in = _B_setup()
    return {'A_x': _A_in['x'], 'A_mem0': _A_in['mem0'], 'A_Wq': _A_in['Wq'], 'A_Wk': _A_in['Wk'], 'A_Wv': _A_in['Wv'], 'A_Wo': _A_in['Wo'], 'A_seg_len': _A_in['seg_len'], 'B_x': _B_in['x'], 'B_w_r': _B_in['w_r'], 'B_w_gate': _B_in['w_gate'], 'B_w_up': _B_in['w_up'], 'B_w_down': _B_in['w_down']}

def reference(A_x, A_mem0, A_Wq, A_Wk, A_Wv, A_Wo, A_seg_len, B_x, B_w_r, B_w_gate, B_w_up, B_w_down):

    def _A_ref(x, mem0, Wq, Wk, Wv, Wo, seg_len):
        B, S, Dm = x.shape
        H, Dh = (Wq.shape[1], Wq.shape[2])
        M = mem0.shape[1]
        scale = Dh ** (-0.5)
        n_seg = S // seg_len
        L = M + seg_len
        idx = jnp.arange(L)
        mask = (idx[:, None] < M) | (idx[:, None] >= idx[None, :])
        mem = mem0
        outs = []
        for s in range(n_seg):
            xs = x[:, s * seg_len:(s + 1) * seg_len, :].copy()
            h = jnp.concatenate([mem, xs], axis=1)
            q = jnp.einsum('btd,dhe->bhte', h, Wq)
            k = jnp.einsum('btd,dhe->bhte', h, Wk)
            v = jnp.einsum('btd,dhe->bhte', h, Wv)
            scores = jnp.einsum('bhqe,bhke->bhqk', q, k) * scale
            scores = jnp.where(mask[None, None], scores, -1000000000.0)
            p = _softmax(scores, axis=-1)
            o = jnp.einsum('bhqk,bhke->bhqe', p, v)
            o = jnp.einsum('bhte,hed->btd', o, Wo)
            mem = o[:, :M, :].copy()
            outs.append(o[:, M:, :])
        return jnp.concatenate(outs, axis=1)

    def _B_ref(x, w_r, w_gate, w_up, w_down):
        B, S, D = x.shape
        C = 8
        r = x @ w_r
        idx = jnp.argsort(-r, axis=-1)[:, :C]
        idx_e = jnp.repeat(idx.reshape(B, C, 1), D, axis=2)
        x_sel = jnp.take_along_axis(x, idx_e, axis=1)
        g = _silu(x_sel @ w_gate)
        u = x_sel @ w_up
        y = g * u @ w_down
        r_sel = _sigmoid(jnp.take_along_axis(r, idx, axis=1))
        y = y * r_sel.reshape(B, C, 1)
        b_off = (jnp.arange(B) * S).reshape(B, 1)
        flat_idx = (idx + b_off).reshape(B * C)
        zero = (x * 0.0).reshape(B * S, D)
        upd = _scatter_add(zero, flat_idx, y.reshape(B * C, D), axis=0)
        return x + upd.reshape(B, S, D)
    x = A_x
    xn = _layernorm(x, axis=-1)
    s = _A_ref(xn, A_mem0, A_Wq, A_Wk, A_Wv, A_Wo, A_seg_len)
    g = _silu(_B_ref(xn, B_w_r, B_w_gate, B_w_up, B_w_down))
    return x + s * g
```

```python
import functools

import jax
import jax.numpy as jnp
import numpy as np
from jax import lax
import jax.experimental.pallas as pl
import jax.experimental.pallas.tpu as pltpu

BF = jnp.bfloat16
F32 = jnp.float32
U32 = jnp.uint32
I32 = jnp.int32

S, D, H, E, M, SEG, FF, C = 2048, 640, 32, 128, 8, 32, 1728, 8
NSEG = S // SEG
RIDE = 24
PRO = 544
EPI0 = 1504
FRONT = 32
LNB = 64
LN0 = 9
NLN = LN0 + 24
TOK = NLN * LNB
QROWS = PRO + RIDE * NSEG
HG = 16
KEY_BIAS = 0x10000000
LN_EPS = 1.0013580322265625e-05
LAG_QK, LAG_PV = 2, 5


def _nn(a, b):
    return lax.dot_general(a, b, (((1,), (0,)), ((), ())), preferred_element_type=F32)


def _nt(a, b):
    return lax.dot_general(a, b, (((1,), (1,)), ((), ())), preferred_element_type=F32)


def _as_bf(x):
    return pltpu.bitcast(x, BF)


def _pack(x):
    return pltpu.bitcast(x.astype(BF), U32)


def _rnd(x):
    return x.astype(BF).astype(F32)


def _silu(x):
    return x * jax.nn.sigmoid(x)


def _cat(xs, axis=0):
    return jnp.concatenate(xs, axis)


def _kernel(x_hbm, mem_hbm, wq_hbm, wk_hbm, wv_hbm, wo_hbm, wr_hbm, wg_hbm, wu_hbm, wd_hbm,
            out_hbm, x_buf, xn_buf, g_buf, wo_buf, mem_buf, q_buf, k_buf, v_buf, w0, w1, w2, w3,
            w4, w5):
    wbufs = (w0, w1, w2, w3, w4, w5)
    dsts = (q_buf, k_buf, v_buf)

    def prologue(st0, st1, st2, st3, st4, st5, xb_buf, wr_buf, wg_buf, wu_buf, wd_buf, key_buf,
                 sel_buf, sems):
        stages = (st0, st1, st2, st3, st4, st5)
        srcs = (wq_hbm, wk_hbm, wv_hbm)
        n0 = LN0 * LNB
        cp_x0 = pltpu.make_async_copy(x_hbm.at[pl.ds(0, n0)], x_buf.at[pl.ds(FRONT, n0)], sems.at[0])
        cp_x1 = pltpu.make_async_copy(x_hbm.at[pl.ds(n0, S - n0)],
                                      x_buf.at[pl.ds(FRONT + n0, S - n0)], sems.at[1])
        cp_wr = pltpu.make_async_copy(wr_hbm, wr_buf, sems.at[2])
        cp_mem = pltpu.make_async_copy(mem_hbm, mem_buf, sems.at[3])
        cp_w = [pltpu.make_async_copy(srcs[c % 3].at[:, pl.ds(HG * (c // 3), HG), :], stages[c],
                                      sems.at[4 + c]) for c in range(6)]
        cp_wo = pltpu.make_async_copy(wo_hbm.bitcast(U32), wo_buf, sems.at[10])
        cp_wg = pltpu.make_async_copy(wg_hbm, wg_buf, sems.at[11])
        cp_wu = pltpu.make_async_copy(wu_hbm, wu_buf, sems.at[12])
        cp_wd = pltpu.make_async_copy(wd_hbm, wd_buf, sems.at[13])
        for cp in (cp_x0, cp_wr, cp_w[0], cp_x1, *cp_w[1:], cp_wg, cp_wu, cp_wd, cp_wo, cp_mem):
            cp.start()

        tail = TOK - S
        x_buf[pl.ds(0, FRONT), :] = jnp.zeros((FRONT, D), BF)
        x_buf[pl.ds(FRONT + S, tail), :] = jnp.zeros((tail, D), BF)
        g_buf[pl.ds(0, FRONT), :] = jnp.zeros((FRONT, D), F32)
        key_buf[...] = jnp.zeros(key_buf.shape, F32)

        def layernorm(blk, keep_bf16):
            t0 = blk * LNB
            if not isinstance(t0, int):
                t0 = pl.multiple_of(t0, LNB)
            x = x_buf[pl.ds(FRONT + t0, LNB), :].astype(F32)
            mean = jnp.sum(x, axis=1, keepdims=True) / D
            cen = x - mean
            var = jnp.sum(cen * cen, axis=1, keepdims=True) / D
            den = _rnd(jnp.sqrt(_rnd(_rnd(var) + LN_EPS)))
            xn = _rnd(_rnd(x - _rnd(mean)) * (1.0 / den))
            xn_buf[pl.ds(t0, LNB), :] = xn
            if keep_bf16:
                xb_buf[pl.ds(t0, LNB), :] = xn.astype(BF)
            g_buf[pl.ds(FRONT + t0, LNB), :] = _rnd(_silu(xn))
            wr = wr_buf[...].astype(F32).reshape(1, D)
            r = _rnd(jnp.sum(xn * wr, axis=1, keepdims=True))
            r = jnp.broadcast_to(r, (LNB, 128))
            bits = lax.shift_right_logical(pltpu.bitcast(r, I32), 16)
            rank = jnp.where(r < 0, 0xFFFF - bits, (bits & 0x7FFF) + 0x8000)
            rank = jnp.where(r != r, 0, rank)
            row = lax.broadcasted_iota(I32, (LNB, 128), 0)
            lane = lax.broadcasted_iota(I32, (LNB, 128), 1)
            tok = row + t0
            key = KEY_BIAS + rank * S + (S - 1 - tok)
            key = jnp.where((row == lane) & (tok < S), key, 0)
            key_buf[pl.ds(blk, 1), :] = jnp.max(pltpu.bitcast(key, F32), axis=0, keepdims=True)

        def relayout(c, d0, nd):
            for j in range(nd // 16):
                d = d0 + 16 * j
                v = pltpu.bitcast(stages[c][pl.ds(d, 16)], U32).reshape(8, 2, HG // 2, 128)
                a = jnp.swapaxes(v[:, 0], 0, 1)
                b = jnp.swapaxes(v[:, 1], 0, 1)
                lo = (a & np.uint32(0xFFFF)) | (b << 16)
                hi = (a >> 16) | (b & np.uint32(0xFFFF0000))
                r = d // 2
                if not isinstance(r, int):
                    r = pl.multiple_of(r, 8)
                for hp in range(HG // 2):
                    wbufs[c][2 * hp, pl.ds(r, 8), :] = lo[hp]
                    wbufs[c][2 * hp + 1, pl.ds(r, 8), :] = hi[hp]

        cp_x0.wait()
        cp_wr.wait()

        def first_ln(i, carry):
            layernorm(i, True)
            return carry

        lax.fori_loop(0, LN0, first_ln, 0)
        cp_w[0].wait()

        def first_relayout(i, carry):
            relayout(0, i * (D // 4), D // 4)
            return carry

        lax.fori_loop(0, 4, first_relayout, 0)
        cp_x1.wait()

        for c in range(6):
            if c < 5:
                cp_w[c + 1].wait()

            def quarter(i, carry, c=c):
                w = _cat([wbufs[c][4 * i + j] for j in range(4)], 1)
                y = _nn(xb_buf[pl.ds(0, PRO), :], _as_bf(w))
                for j in range(4):
                    dsts[c % 3][HG * (c // 3) + 4 * i + j, pl.ds(0, PRO // 2), :] = _pack(
                        y[:, j * E:(j + 1) * E])
                if c < 5:
                    relayout(c + 1, i * (D // 4), D // 4)
                layernorm(LN0 + 4 * c + i, False)
                return carry

            lax.fori_loop(0, 4, quarter, 0)

        keys = key_buf[...]
        crow = lax.broadcasted_iota(I32, (C, 128), 0)
        top = jnp.zeros((C, 128), I32)
        idxs = []
        for c in range(C):
            kmax = jnp.max(jnp.max(keys, axis=0, keepdims=True), axis=1, keepdims=True)
            keys = jnp.where(keys == kmax, 0.0, keys)
            kbits = pltpu.bitcast(jnp.broadcast_to(kmax, (C, 128)), I32)
            top = jnp.where(crow == c, kbits, top)
            idx = jnp.max((S - 1 - (kbits & (S - 1))).astype(F32)).astype(I32)
            idx = jnp.clip(idx, 0, S - 1)
            idxs.append(idx)
            sel_buf[pl.ds(c, 1), :] = xn_buf[pl.ds(idx, 1), :]
        rank = lax.shift_right_logical(top - KEY_BIAS, 11)
        rbits = jnp.where(rank >= 0x8000, rank - 0x8000, 0xFFFF - rank)
        r_sel = pltpu.bitcast(rbits << 16, F32)[:, 0:1]
        cp_wg.wait()
        cp_wu.wait()
        cp_wd.wait()
        xs = sel_buf[...]
        gate = _rnd(_silu(_rnd(_nt(xs, wg_buf[...]))))
        up = _rnd(_nt(xs, wu_buf[...]))
        y = _rnd(_nn(_rnd(gate * up), wd_buf[...]))
        y = _rnd(y * _rnd(jax.nn.sigmoid(r_sel)))
        g_sel = _rnd(_silu(_rnd(xs + y)))
        for c in range(C):
            g_buf[pl.ds(FRONT + idxs[c], 1), :] = g_sel[c:c + 1]
        cp_wo.wait()
        cp_mem.wait()

    pl.run_scoped(
        prologue,
        *[pltpu.VMEM((D, HG, E), BF) for _ in range(6)],
        pltpu.VMEM((LN0 * LNB, D), BF),
        pltpu.VMEM((D,), BF),
        pltpu.VMEM((FF, D), BF),
        pltpu.VMEM((FF, D), BF),
        pltpu.VMEM((FF, D), BF),
        pltpu.VMEM((40, 128), F32),
        pltpu.VMEM((C, D), F32),
        pltpu.SemaphoreType.DMA((14,)),
    )

    def scan(o_buf, out_buf, sems):
        o_buf[:, pl.ds(0, FRONT // 2), :] = jnp.zeros((H, FRONT // 2, E), U32)
        nk = SEG + 16
        row = lax.broadcasted_iota(I32, (SEG, nk), 0)
        col = lax.broadcasted_iota(I32, (SEG, nk), 1)
        x_mask = (col <= row) | ((col >= SEG) & (col < SEG + M))
        x_fill = jnp.where(col < SEG + M, -1e9, -jnp.inf).astype(F32)
        m_mask = lax.broadcasted_iota(I32, (M, nk), 1) < SEG + M
        zeros = jnp.zeros((M, E), F32)
        scale = E ** -0.5

        def softmax(s, mask, fill):
            s = jnp.where(mask, s * scale, fill)
            e = jnp.exp(s - jnp.max(s, axis=1, keepdims=True))
            return e / jnp.sum(e, axis=1, keepdims=True)

        def finish(r, n, s):
            x = x_buf[pl.ds(r, n), :].astype(F32)
            out_buf[pl.ds(r, n), :] = (x + _rnd(_rnd(s) * g_buf[pl.ds(r, n), :])).astype(BF)

        def step(i, par, mem):
            s = 2 * i + par
            seg = pl.multiple_of(s * (SEG // 2), SEG // 2)
            rin = pl.multiple_of(PRO + RIDE * s, 8)
            win = pl.multiple_of(PRO // 2 + RIDE * i + 8 * par, 8)
            wout = pl.multiple_of(RIDE * i + 16 * par, 8)
            lhs = _cat([mem, xn_buf[pl.ds(rin, RIDE), :]]).astype(BF)
            qm, qx, kc, vc, pm, px, om, ride, acc = {}, {}, {}, {}, {}, {}, {}, {}, []

            def put(ref, h, y):
                if par == 0:
                    ref[h, pl.ds(win, 8), :] = _pack(y[8:24])
                    ref[h, pl.ds(win + 8, 4), :] = _pack(y[16:32])[4:8]
                else:
                    ref[h, pl.ds(win + 4, 4), :] = _pack(y[0:16])[4:8]
                    ref[h, pl.ds(win + 8, 8), :] = _pack(y[16:32])

            def qkv(h):
                g, hh = divmod(h, HG)
                kx = k_buf[h, pl.ds(seg, SEG // 2), :]
                vx = v_buf[h, pl.ds(seg, SEG // 2), :]
                qx[h] = _as_bf(q_buf[h, pl.ds(seg, SEG // 2), :])
                y = _nn(lhs, _as_bf(_cat([wbufs[3 * g + m][hh] for m in range(3)], 1)))
                q, k, v = y[:, 0:E], y[:, E:2 * E], y[:, 2 * E:3 * E]
                put(q_buf, h, q)
                put(k_buf, h, k)
                put(v_buf, h, v)
                qm[h] = _rnd(q[0:M])
                kc[h] = _as_bf(_cat([kx, _pack(_cat([k[0:M], zeros]))]))
                vc[h] = _as_bf(_cat([vx, _pack(_cat([v[0:M], zeros]))]))

            def qk_m(h):
                pm[h] = _rnd(softmax(_nt(qm[h], kc[h]), m_mask, -jnp.inf))

            def qk_x(h):
                px[h] = softmax(_nt(qx[h], kc[h]), x_mask, x_fill).astype(BF)

            def pv_m(h):
                om[h] = _nn(pm[h], vc[h])

            def pv_x(h):
                o_buf[h, pl.ds(seg + FRONT // 2, SEG // 2), :] = _pack(_nn(px[h], vc[h]))

            def proj(h):
                full, half = ride[h]
                o = _as_bf(_cat([_pack(_cat([om[h], half])), full]))
                y = _nn(o, _as_bf(wo_buf[h]))
                acc[:] = [y if not acc else acc[0] + y]

            for h in range(H):
                w0_ = o_buf[h, pl.ds(wout, 8), :]
                w1_ = o_buf[h, pl.ds(wout + 8, 8), :]
                if par == 0:
                    ride[h] = (w1_, _as_bf(w0_).astype(F32)[8:16])
                else:
                    ride[h] = (w0_, _as_bf(w1_).astype(F32)[0:8])

            order = [(15 * h, 0, qkv, h) for h in range(H)]
            order += [(15 * H + 5 * h, 0, proj, h) for h in range(H)]
            for h in range(H):
                order.append((15 * (h + LAG_QK) - 0.5, 1, qk_m, h))
                order.append((15 * (h + LAG_QK) - 0.4, 1, qk_x, h))
                order.append((15 * (h + LAG_PV) - 0.5, 2, pv_m, h))
                order.append((15 * (h + LAG_PV) - 0.4, 2, pv_x, h))
            order.sort(key=lambda e: e[:2])
            for _, _, fn, h in order:
                fn(h)

            y = acc[0]
            rout = pl.multiple_of(RIDE * s + FRONT - RIDE, 8)
            finish(rout, RIDE, y[8:32] if par == 0 else _cat([y[16:32], y[8:16]]))
            return _rnd(y[0:M])

        def two_steps(i, mem):
            return step(i, 1, step(i, 0, mem))

        lax.fori_loop(0, NSEG // 2, two_steps, mem_buf[...].astype(F32))

        copies = [pltpu.make_async_copy(out_buf.at[pl.ds(FRONT, EPI0)], out_hbm.at[pl.ds(0, EPI0)],
                                        sems.at[0])]
        copies[0].start()
        t = EPI0
        for b, n in enumerate((144, 144, 128, 128)):
            o = _as_bf(_cat([o_buf[h, pl.ds((FRONT + t) // 2, n // 2), :] for h in range(H)], 1))
            w = _as_bf(wo_buf[...].reshape(H * E // 2, D))
            finish(FRONT + t, n, _nn(o, w))
            copies.append(pltpu.make_async_copy(out_buf.at[pl.ds(FRONT + t, n)],
                                                out_hbm.at[pl.ds(t, n)], sems.at[1 + b]))
            copies[-1].start()
            t += n
        for cp in copies:
            cp.wait()

    pl.run_scoped(
        scan,
        pltpu.VMEM((H, (FRONT + S) // 2, E), U32),
        pltpu.VMEM((FRONT + S, D), BF),
        pltpu.SemaphoreType.DMA((5,)),
    )


@functools.partial(jax.jit, static_argnames=("A_seg_len",))
def pallas_recurrent_scan__memory_aug_recurrent_mem_tr__moe_arch_mod__prompt_kernel(
    A_x: jax.Array,
    A_mem0: jax.Array,
    A_Wq: jax.Array,
    A_Wk: jax.Array,
    A_Wv: jax.Array,
    A_Wo: jax.Array,
    A_seg_len: int,
    B_x: jax.Array,
    B_w_r: jax.Array,
    B_w_gate: jax.Array,
    B_w_up: jax.Array,
    B_w_down: jax.Array,
):
    del B_x
    assert A_seg_len == SEG and A_x.shape == (1, S, D) and A_mem0.shape == (1, M, D)
    assert A_Wq.shape == (D, H, E) and A_Wo.shape == (H, E, D) and B_w_gate.shape == (D, FF)
    hbm = pl.BlockSpec(memory_space=pltpu.MemorySpace.HBM)
    out = pl.pallas_call(
        _kernel,
        out_shape=jax.ShapeDtypeStruct((S, D), BF),
        in_specs=[hbm] * 10,
        out_specs=hbm,
        scratch_shapes=[
            pltpu.VMEM((FRONT + TOK, D), BF),
            pltpu.VMEM((TOK, D), F32),
            pltpu.VMEM((FRONT + TOK, D), F32),
            pltpu.VMEM((H, E // 2, D), U32),
            pltpu.VMEM((M, D), BF),
            *[pltpu.VMEM((H, QROWS // 2, E), U32) for _ in range(3)],
            *[pltpu.VMEM((HG, D // 2, E), U32) for _ in range(6)],
        ],
        compiler_params=pltpu.CompilerParams(vmem_limit_bytes=124 * 1024 * 1024),
    )(A_x.reshape(S, D), A_mem0.reshape(M, D), A_Wq, A_Wk, A_Wv, A_Wo, B_w_r, B_w_gate.T, B_w_up.T,
      B_w_down)
    return out.reshape(1, S, D)
```

```python
import functools

import jax
import jax.numpy as jnp
import numpy as np
from jax import lax
import jax.experimental.pallas as pl
import jax.experimental.pallas.tpu as pltpu

BF = jnp.bfloat16
F32 = jnp.float32
U32 = jnp.uint32
I32 = jnp.int32

S, D, H, E, M, SEG, FF, C = 2048, 640, 32, 128, 8, 32, 1728, 8
NSEG = S // SEG
RIDE = 24
PRO = 544
EPI0 = 1504
FRONT = 32
LNB = 128
LNP = 32
LN0 = 576
TOK = LN0 + 12 * LNB
PRO_BLOCKS = (144, 144, 128, 128)
A_XN, A_G, A_XB = 0, TOK + FRONT, TOK + FRONT + S
QROWS = PRO + RIDE * NSEG
HG = 16
KEY_BIAS = 0x10000000
LOG2E = 1.4426950408889634
LN_EPS = 1.0013580322265625e-05
LAG_QK, LAG_PV = 4, 8
ONLY_MAIN = False
NG = 4
NGO = 1
MASKED = 0
KMAJOR = 1
PLAN = 0
LQ, LP, LQM, LPM = 4, 8, 4, 8
OQ, OP, OQM, OPM = 1, 2, 2, 1
TAILX = 16
ANCHOR = 3


def _nn(a, b):
    return lax.dot_general(a, b, (((1,), (0,)), ((), ())), preferred_element_type=F32)


def _nt(a, b):
    return lax.dot_general(a, b, (((1,), (1,)), ((), ())), preferred_element_type=F32)


def _as_bf(x):
    return pltpu.bitcast(x, BF)


def _pack(x):
    return pltpu.bitcast(x.astype(BF), U32)


def _rnd(x):
    return x.astype(BF).astype(F32)


def _silu(x):
    return x * jax.nn.sigmoid(x)


def _recip(x):
    r = pl.reciprocal(x, approx=True)
    return r * (2.0 - x * r)


def _silu_bounded(x):
    return x * _recip(1.0 + jnp.exp(-x))


def _cat(xs, axis=0):
    return jnp.concatenate(xs, axis)


def _interleave(*gens):
    gens = list(gens)
    while gens:
        gens = [g for g in gens if next(g, StopIteration) is not StopIteration]


def _kernel(x_hbm, mem_hbm, wq_hbm, wk_hbm, wv_hbm, wo_hbm, wr_hbm, wg_hbm, wu_hbm, wd_hbm,
            out_hbm, x_buf, act_buf, wo_buf, mem_buf, *bufs):
    w_buf = bufs[0]
    qkv_bufs = bufs[1:]

    def act(base, r, n):
        return pltpu.bitcast(act_buf[pl.ds(base + r, n), :], F32)

    def set_act(base, r, val):
        act_buf[pl.ds(base + r, val.shape[0]), :] = pltpu.bitcast(val, U32)

    def prologue(wr_buf, wg_buf, wu_buf, wd_buf, key_buf, sel_buf, sems, wsems):
        srcs = [w.bitcast(U32) for w in (wq_hbm, wk_hbm, wv_hbm)]
        n0 = LN0
        cp_x0 = pltpu.make_async_copy(x_hbm.at[pl.ds(0, n0)], x_buf.at[pl.ds(FRONT, n0)], sems.at[0])
        cp_x1 = pltpu.make_async_copy(x_hbm.at[pl.ds(n0, S - n0)],
                                      x_buf.at[pl.ds(FRONT + n0, S - n0)], sems.at[1])
        cp_wr = pltpu.make_async_copy(wr_hbm, wr_buf, sems.at[2])
        cp_mem = pltpu.make_async_copy(mem_hbm, mem_buf, sems.at[3])

        def weight_copies(j, m):
            src_j = min(j, H // 4 - 1) if isinstance(j, int) else jnp.minimum(j, H // 4 - 1)
            return [pltpu.make_async_copy(srcs[m].at[:, t % 2, 2 * src_j + t // 2, :],
                                          w_buf.at[4 * (3 * j + m) + t], wsems.at[3 * j + m])
                    for t in range(4)]

        cp_wo = pltpu.make_async_copy(wo_hbm.bitcast(U32), wo_buf, sems.at[4])
        cp_wg = pltpu.make_async_copy(wg_hbm, wg_buf, sems.at[5])
        cp_wu = pltpu.make_async_copy(wu_hbm, wu_buf, sems.at[6])
        cp_wd = pltpu.make_async_copy(wd_hbm, wd_buf, sems.at[7])
        def start_weights(j):
            for jm in ((j, 1), (j, 2), (j + 1, 0)):
                for cp in weight_copies(*jm):
                    cp.start()

        for cp in (cp_x0, cp_wr, *weight_copies(0, 0)):
            cp.start()

        tail = TOK - S
        x_buf[pl.ds(0, FRONT), :] = jnp.zeros((FRONT, D), BF)
        x_buf[pl.ds(FRONT + S, tail), :] = jnp.zeros((tail, D), BF)
        set_act(A_G - FRONT, 0, jnp.zeros((FRONT, D), F32))

        def layernorm(t0, n, packed):
            x = x_buf[pl.ds(FRONT + t0, n), :].astype(F32)
            mean = jnp.sum(x, axis=1, keepdims=True) / D
            cen = x - mean
            var = jnp.sum(cen * cen, axis=1, keepdims=True) / D
            den = _rnd(jnp.sqrt(_rnd(_rnd(var) + LN_EPS)))
            xn = _rnd(_rnd(x - _rnd(mean)) * (1.0 / den))
            set_act(A_XN, t0, xn)
            if packed:
                act_buf[pl.ds(pl.multiple_of(A_XB + t0 // 2, 8), n // 2), :] = _pack(xn)

        def layernorm_pieces(t0):
            for p in range(4):
                layernorm(pl.multiple_of(t0 + p * (LNB // 2), LNB // 2), LNB // 2, False)
                yield

        def gate_pieces(blk):
            wr = wr_buf[...].astype(F32).reshape(1, D)
            best = None
            for p in range(LNB // LNP):
                t0 = pl.multiple_of(blk * LNB + p * LNP, LNP)
                xn = act(A_XN, t0, LNP)
                set_act(A_G, t0, _rnd(_silu_bounded(xn)))
                r = _rnd(jnp.sum(xn * wr, axis=1, keepdims=True))
                r = jnp.broadcast_to(r, (LNP, 128))
                bits = lax.shift_right_logical(pltpu.bitcast(r, I32), 16)
                rank = jnp.where(r < 0, 0xFFFF - bits, (bits & 0x7FFF) + 0x8000)
                rank = jnp.where(r != r, 0, rank)
                row = lax.broadcasted_iota(I32, (LNP, 128), 0) + p * LNP
                lane = lax.broadcasted_iota(I32, (LNP, 128), 1)
                key = KEY_BIAS + rank * S + (S - 1 - blk * LNB - lane)
                key = pltpu.bitcast(jnp.where(row == lane, key, 0), F32)
                best = key if best is None else jnp.maximum(best, key)
                yield
            key_buf[pl.ds(blk, 1), :] = jnp.max(best, axis=0, keepdims=True)

        def unzip_pieces(u):
            for t in (0, 2):
                for r in range(0, D // 2, D // 4):
                    rows = pl.ds(r, D // 4)
                    a = w_buf[4 * u + t, rows, :]
                    b = w_buf[4 * u + t + 1, rows, :]
                    w_buf[4 * u + t, rows, :] = (a & np.uint32(0xFFFF)) | (b << 16)
                    w_buf[4 * u + t + 1, rows, :] = (a >> 16) | (b & np.uint32(0xFFFF0000))
                    yield

        def project_pieces(j, m, odd):
            r0 = 0
            for n in PRO_BLOCKS:
                w = _cat([w_buf[4 * (3 * j + m) + t] for t in range(4)], 1)
                y = _nn(_as_bf(act_buf[pl.ds(A_XB + r0, n // 2), :]), _as_bf(w))
                for t in range(4):
                    qkv_bufs[2 * m + odd][4 * (j // 2) + t, pl.ds(r0, n // 2), :] = _pack(
                        y[:, t * E:(t + 1) * E])
                r0 += n // 2
                yield

        cp_x0.wait()
        cp_wr.wait()
        start_weights(0)

        def first_ln(i, carry):
            layernorm(pl.multiple_of(i * (LN0 // 3), LN0 // 3), LN0 // 3, True)
            return carry

        lax.fori_loop(0, 3, first_ln, 0)
        for cp in weight_copies(0, 0):
            cp.wait()
        _interleave(unzip_pieces(0))

        def two_quads(i, carry):
            for odd in range(2):
                j = 2 * i + odd
                for jm in ((j, 1), (j, 2), (j + 1, 0)):
                    for cp in weight_copies(*jm):
                        cp.wait()
                if odd:
                    pl.when(i == 0)(cp_x1.wait)
                    pl.when(i < H // 8 - 1)(functools.partial(start_weights, j + 1))
                    for k, cp in enumerate((cp_wo, cp_wu, cp_mem)):
                        pl.when(i == k)(cp.start)
                else:
                    start_weights(j + 1)
                    for k, cp in enumerate((cp_x1, cp_wg, cp_wd)):
                        pl.when(i == k)(cp.start)
                t0 = jnp.clip(LN0 + (j - 1) * 2 * LNB, LN0 - 2 * LNB, TOK - 2 * LNB)
                for m in range(3):
                    side = gate_pieces(2 * j + m) if m < 2 else layernorm_pieces(t0)
                    _interleave(project_pieces(j, m, odd), unzip_pieces(3 * j + m + 1), side)
            return carry

        lax.fori_loop(0, H // 8, two_quads, 0)

        keys = key_buf[...]
        crow = lax.broadcasted_iota(I32, (C, 128), 0)
        top = jnp.zeros((C, 128), I32)
        idxs = []
        for c in range(C):
            kmax = jnp.max(jnp.max(keys, axis=0, keepdims=True), axis=1, keepdims=True)
            keys = jnp.where(keys == kmax, 0.0, keys)
            kbits = pltpu.bitcast(jnp.broadcast_to(kmax, (C, 128)), I32)
            top = jnp.where(crow == c, kbits, top)
            idx = jnp.max((S - 1 - (kbits & (S - 1))).astype(F32)).astype(I32)
            idx = jnp.clip(idx, 0, S - 1)
            idxs.append(idx)
            sel_buf[pl.ds(c, 1), :] = act_buf[pl.ds(A_XN + idx, 1), :]
        rank = lax.shift_right_logical(top - KEY_BIAS, 11)
        rbits = jnp.where(rank >= 0x8000, rank - 0x8000, 0xFFFF - rank)
        r_sel = pltpu.bitcast(rbits << 16, F32)[:, 0:1]
        cp_wg.wait()
        cp_wu.wait()
        cp_wd.wait()
        xs = pltpu.bitcast(sel_buf[...], F32)
        gate = _rnd(_silu(_rnd(_nt(xs, wg_buf[...]))))
        up = _rnd(_nt(xs, wu_buf[...]))
        y = _rnd(_nn(_rnd(gate * up), wd_buf[...]))
        y = _rnd(y * _rnd(jax.nn.sigmoid(r_sel)))
        g_sel = pltpu.bitcast(_rnd(_silu(_rnd(xs + y))), U32)
        for c in range(C):
            act_buf[pl.ds(A_G + idxs[c], 1), :] = g_sel[c:c + 1]
        cp_wo.wait()
        cp_mem.wait()

    if not ONLY_MAIN: pl.run_scoped(
        prologue,
        pltpu.VMEM((D,), BF),
        pltpu.VMEM((FF, D), BF),
        pltpu.VMEM((FF, D), BF),
        pltpu.VMEM((FF, D), BF),
        pltpu.VMEM((S // LNB, 128), F32),
        pltpu.VMEM((C, D), U32),
        pltpu.SemaphoreType.DMA((8,)),
        pltpu.SemaphoreType.DMA((3 * (H // 4) + 1,)),
    )

    def scan(out_buf, sems, px_buf, pm_buf, qm_buf, km_buf, vm_buf, om_buf, *o_bufs):
        for o_buf in o_bufs:
            o_buf[:, pl.ds(0, FRONT // 2), :] = jnp.zeros((H // NGO, FRONT // 2, E), U32)
        nk = SEG + 16
        row = lax.broadcasted_iota(I32, (SEG, nk), 0)
        col = lax.broadcasted_iota(I32, (SEG, nk), 1)
        x_mask = (col <= row) | ((col >= SEG) & (col < SEG + M))
        x_fill = jnp.where(col < SEG + M, -1e9 * LOG2E, -jnp.inf).astype(F32)
        m_mask = lax.broadcasted_iota(I32, (M, nk), 1) < SEG + M
        zeros = jnp.zeros((M, E), F32)

        def softmax(s, mask, fill):
            s = jnp.where(mask, s * (E ** -0.5 * LOG2E), fill)
            e = jnp.exp2(s - jnp.max(s, axis=1, keepdims=True))
            l = jnp.sum(e, axis=1, keepdims=True)
            return e * _recip(l)

        def finish(r, n, s):
            x = x_buf[pl.ds(r, n), :].astype(F32)
            out_buf[pl.ds(r, n), :] = (x + _rnd(_rnd(s) * act(A_G - FRONT, r, n))).astype(BF)

        def step(i, par, mem):
            s = 2 * i + par
            seg = pl.multiple_of(s * (SEG // 2), SEG // 2)
            rin = pl.multiple_of(PRO + RIDE * s, 8)
            win = pl.multiple_of(PRO // 2 + RIDE * i + 8 * par, 8)
            wout = pl.multiple_of(RIDE * i + 16 * par, 8)
            lhs = _cat([mem, act(A_XN, rin, RIDE)]).astype(BF)
            qm, qx, kc, vc, pm, px, om, ride, acc = {}, {}, {}, {}, {}, {}, {}, {}, []
            keep = lax.broadcasted_iota(I32, (8, E), 1) < E + (i >> 10)

            def park(ref, h, val):
                if MASKED:
                    pltpu.store(ref.at[h], val, mask=keep)
                else:
                    ref[h] = val

            def at(m, h, start, n):
                if m == 3:
                    return o_bufs[h % NGO].at[h // NGO, pl.ds(start, n), :]
                j, t = divmod(h, 4)
                return qkv_bufs[2 * m + j % 2].at[4 * (j // 2) + t, pl.ds(start, n), :]

            def put(bufs_, h, y):
                if par == 0:
                    at(bufs_, h, win, 8)[...] = _pack(y[8:24])
                    at(bufs_, h, win + 8, 4)[...] = _pack(y[16:32])[4:8]
                else:
                    at(bufs_, h, win + 4, 4)[...] = _pack(y[0:16])[4:8]
                    at(bufs_, h, win + 8, 8)[...] = _pack(y[16:32])

            def rnd(arg):
                j, m = arg
                w = _as_bf(_cat([w_buf[4 * (3 * j + m) + t] for t in range(4)], 1))
                if KMAJOR:
                    y = None
                    for kk in range(D // E):
                        z = _nn(lhs[:, kk * E:(kk + 1) * E], w[kk * E:(kk + 1) * E])
                        y = z if y is None else y + z
                else:
                    y = _nn(lhs, w)
                for t in range(4):
                    h = 4 * j + t
                    yh = y[:, t * E:(t + 1) * E]
                    put(m, h, yh)
                    if m == 0:
                        qm[h] = _rnd(yh[0:M])
                    elif m == 1:
                        kc[h] = _pack(_cat([yh[0:M], zeros]))
                    else:
                        vc[h] = _pack(_cat([yh[0:M], zeros]))

            def keys(h):
                return _as_bf(_cat([at(1, h, seg, SEG // 2)[...], km_buf[h] if ANCHOR & 4 else kc[h]]))

            def vals(h):
                return _as_bf(_cat([at(2, h, seg, SEG // 2)[...], vm_buf[h] if ANCHOR & 4 else vc[h]]))

            def qk_m(h):
                pm[h] = _rnd(softmax(_nt(qm_buf[h] if ANCHOR & 4 else qm[h], keys(h)), m_mask, -jnp.inf))
                if ANCHOR & 1:
                    pm_buf[h] = pm[h]

            def qk_x(h):
                q = _as_bf(at(0, h, seg, SEG // 2)[...])
                px[h] = softmax(_nt(q, keys(h)), x_mask, x_fill).astype(BF)
                if ANCHOR & 2:
                    px_buf[h] = px[h]

            def pv_m(h):
                om[h] = _nn(pm_buf[h] if ANCHOR & 1 else pm[h], vals(h))
                if ANCHOR & 8:
                    park(om_buf, h, om[h])

            def pv_x(h):
                o = _nn(px_buf[h] if ANCHOR & 2 else px[h], vals(h))
                at(3, h, seg + FRONT // 2, SEG // 2)[...] = _pack(o)

            def proj(h):
                w0_ = at(3, h, wout, 8)[...]
                w1_ = at(3, h, wout + 8, 8)[...]
                if par == 0:
                    full, half = w1_, _as_bf(w0_).astype(F32)[8:16]
                else:
                    full, half = w0_, _as_bf(w1_).astype(F32)[0:8]
                o = _as_bf(_cat([_pack(_cat([om_buf[h] if ANCHOR & 8 else om[h], half])), full]))
                y = _nn(o, _as_bf(wo_buf[h]))
                acc[:] = [y if not acc else acc[0] + y]

            order = [(3 * j + m, 0, rnd, (j, m)) for j in range(H // 4) for m in range(3)]
            order += [(24 + h / 4, 0, proj, h) for h in range(H)]
            for h in range(H):
                j, t = divmod(h, 4)
                order.append((3 * j + LQM - 0.5, OQM, qk_m, h))
                order.append((3 * j + LQ - 0.5, OQ, qk_x, h))
                order.append((3 * j + LPM - 0.5, OPM, pv_m, h))
                order.append((3 * j + LP - 0.5 if h < H - TAILX else 1000, OP, pv_x, h))
            order.sort(key=lambda e: e[:2])
            for _, _, fn, h in order:
                fn(h)

            y = acc[0]
            rout = pl.multiple_of(RIDE * s + FRONT - RIDE, 8)
            finish(rout, RIDE, y[8:32] if par == 0 else _cat([y[16:32], y[8:16]]))
            return _rnd(y[0:M])

        def two_steps(i, mem):
            return step(i, 1, step(i, 0, mem))

        lax.fori_loop(0, NSEG // 2, two_steps, mem_buf[...].astype(F32))

        copies = [pltpu.make_async_copy(out_buf.at[pl.ds(FRONT, EPI0)], out_hbm.at[pl.ds(0, EPI0)],
                                        sems.at[0])]
        copies[0].start()
        t = EPI0
        for b, n in enumerate((144, 144, 128, 128) if not ONLY_MAIN else ()):
            o = _as_bf(_cat([o_bufs[h % NGO][h // NGO, pl.ds((FRONT + t) // 2, n // 2), :] for h in range(H)], 1))
            w = _as_bf(wo_buf[...].reshape(H * E // 2, D))
            finish(FRONT + t, n, _nn(o, w))
            copies.append(pltpu.make_async_copy(out_buf.at[pl.ds(FRONT + t, n)],
                                                out_hbm.at[pl.ds(t, n)], sems.at[1 + b]))
            copies[-1].start()
            t += n
        for cp in copies:
            cp.wait()

    pl.run_scoped(
        scan,
        pltpu.VMEM((FRONT + S, D), BF),
        pltpu.SemaphoreType.DMA((5,)),
        pltpu.VMEM((H, SEG, SEG + 16), BF),
        pltpu.VMEM((H, M, SEG + 16), F32),
        pltpu.VMEM((H, M, E), F32),
        pltpu.VMEM((H, 8, E), U32),
        pltpu.VMEM((H, 8, E), U32),
        pltpu.VMEM((H, M, E), F32),
        *[pltpu.VMEM((H // NGO, (FRONT + S) // 2, E), U32) for _ in range(NGO)],
    )


@functools.partial(jax.jit, static_argnames=("A_seg_len",))
def pallas_recurrent_scan__memory_aug_recurrent_mem_tr__moe_arch_mod__prompt_kernel(
    A_x: jax.Array,
    A_mem0: jax.Array,
    A_Wq: jax.Array,
    A_Wk: jax.Array,
    A_Wv: jax.Array,
    A_Wo: jax.Array,
    A_seg_len: int,
    B_x: jax.Array,
    B_w_r: jax.Array,
    B_w_gate: jax.Array,
    B_w_up: jax.Array,
    B_w_down: jax.Array,
):
    del B_x
    assert A_seg_len == SEG and A_x.shape == (1, S, D) and A_mem0.shape == (1, M, D)
    assert A_Wq.shape == (D, H, E) and A_Wo.shape == (H, E, D) and B_w_gate.shape == (D, FF)
    hbm = pl.BlockSpec(memory_space=pltpu.MemorySpace.HBM)
    out = pl.pallas_call(
        _kernel,
        out_shape=jax.ShapeDtypeStruct((S, D), BF),
        in_specs=[hbm] * 10,
        out_specs=hbm,
        scratch_shapes=[
            pltpu.VMEM((FRONT + TOK, D), BF),
            pltpu.VMEM((A_XB + LN0 // 2, D), U32),
            pltpu.VMEM((H, E // 2, D), U32),
            pltpu.VMEM((M, D), BF),
            pltpu.VMEM((3 * H + 4, D // 2, E), U32),
            *[pltpu.VMEM((H // 2, QROWS // 2, E), U32) for _ in range(6)],
        ],
        compiler_params=pltpu.CompilerParams(vmem_limit_bytes=124 * 1024 * 1024),
    )(A_x.reshape(S, D), A_mem0.reshape(M, D),
      *(w.reshape(D // 2, 2, H, E) for w in (A_Wq, A_Wk, A_Wv)), A_Wo, B_w_r, B_w_gate.T, B_w_up.T,
      B_w_down)
    return out.reshape(1, S, D)
```

```python
import functools

import jax
import jax.numpy as jnp
import numpy as np
from jax import lax
import jax.experimental.pallas as pl
import jax.experimental.pallas.tpu as pltpu

BF = jnp.bfloat16
F32 = jnp.float32
U32 = jnp.uint32
I32 = jnp.int32

S, D, H, E, M, SEG, FF, C = 2048, 640, 32, 128, 8, 32, 1728, 8
NSEG = S // SEG
RIDE = 24
PRO = 544
EPI0 = 1504
FRONT = 32
LNB = 128
LNP = 32
LN0 = 576
TOK = LN0 + 12 * LNB
PRO_BLOCKS = (144, 144, 128, 128)
A_XN, A_G, A_XB = 0, TOK + FRONT, TOK + FRONT + S
QROWS = PRO + RIDE * NSEG
HG = 16
KEY_BIAS = 0x10000000
LOG2E = 1.4426950408889634
LN_EPS = 1.0013580322265625e-05
LAG_QK, LAG_PV = 4, 8
ONLY_MAIN = False
MERGE_QK, MERGE_PV, UNROLL, HALF = 1, 1, 2, 0
NG = 4
NGO = 1
MASKED = 0
KMAJOR = 1
PLAN = 0
LQ, LP, LQM, LPM = 4, 8, 4, 7
OQ, OP, OQM, OPM = 1, 2, 2, 1
TAILX = 12
ANCHOR = 3


def _nn(a, b):
    return lax.dot_general(a, b, (((1,), (0,)), ((), ())), preferred_element_type=F32)


def _nt(a, b):
    return lax.dot_general(a, b, (((1,), (1,)), ((), ())), preferred_element_type=F32)


def _as_bf(x):
    return pltpu.bitcast(x, BF)


def _pack(x):
    return pltpu.bitcast(x.astype(BF), U32)


def _rnd(x):
    return x.astype(BF).astype(F32)


def _silu(x):
    return x * jax.nn.sigmoid(x)


def _recip(x):
    r = pl.reciprocal(x, approx=True)
    return r * (2.0 - x * r)


def _silu_bounded(x):
    return x * _recip(1.0 + jnp.exp(-x))


def _cat(xs, axis=0):
    return jnp.concatenate(xs, axis)


def _interleave(*gens):
    gens = list(gens)
    while gens:
        gens = [g for g in gens if next(g, StopIteration) is not StopIteration]


def _kernel(x_hbm, mem_hbm, wq_hbm, wk_hbm, wv_hbm, wo_hbm, wr_hbm, wg_hbm, wu_hbm, wd_hbm,
            out_hbm, x_buf, act_buf, wo_buf, mem_buf, *bufs):
    w_buf = bufs[0]
    qkv_bufs = [b.bitcast(BF) for b in bufs[1:]]

    def act(base, r, n):
        return pltpu.bitcast(act_buf[pl.ds(base + r, n), :], F32)

    def set_act(base, r, val):
        act_buf[pl.ds(base + r, val.shape[0]), :] = pltpu.bitcast(val, U32)

    def prologue(wr_buf, wg_buf, wu_buf, wd_buf, key_buf, sel_buf, sems, wsems):
        srcs = [w.bitcast(U32) for w in (wq_hbm, wk_hbm, wv_hbm)]
        n0 = LN0
        cp_x0 = pltpu.make_async_copy(x_hbm.at[pl.ds(0, n0)], x_buf.at[pl.ds(FRONT, n0)], sems.at[0])
        cp_x1 = pltpu.make_async_copy(x_hbm.at[pl.ds(n0, S - n0)],
                                      x_buf.at[pl.ds(FRONT + n0, S - n0)], sems.at[1])
        cp_wr = pltpu.make_async_copy(wr_hbm, wr_buf, sems.at[2])
        cp_mem = pltpu.make_async_copy(mem_hbm, mem_buf, sems.at[3])

        def weight_copies(j, m):
            src_j = min(j, H // 4 - 1) if isinstance(j, int) else jnp.minimum(j, H // 4 - 1)
            return [pltpu.make_async_copy(srcs[m].at[:, t % 2, 2 * src_j + t // 2, :],
                                          w_buf.at[4 * (3 * j + m) + t], wsems.at[3 * j + m])
                    for t in range(4)]

        cp_wo = pltpu.make_async_copy(wo_hbm.bitcast(U32), wo_buf, sems.at[4])
        cp_wg = pltpu.make_async_copy(wg_hbm, wg_buf, sems.at[5])
        cp_wu = pltpu.make_async_copy(wu_hbm, wu_buf, sems.at[6])
        cp_wd = pltpu.make_async_copy(wd_hbm, wd_buf, sems.at[7])
        def start_weights(j):
            for jm in ((j, 1), (j, 2), (j + 1, 0)):
                for cp in weight_copies(*jm):
                    cp.start()

        for cp in (cp_x0, cp_wr, *weight_copies(0, 0)):
            cp.start()

        tail = TOK - S
        x_buf[pl.ds(0, FRONT), :] = jnp.zeros((FRONT, D), BF)
        x_buf[pl.ds(FRONT + S, tail), :] = jnp.zeros((tail, D), BF)
        set_act(A_G - FRONT, 0, jnp.zeros((FRONT, D), F32))

        def layernorm(t0, n, packed):
            x = x_buf[pl.ds(FRONT + t0, n), :].astype(F32)
            mean = jnp.sum(x, axis=1, keepdims=True) / D
            cen = x - mean
            var = jnp.sum(cen * cen, axis=1, keepdims=True) / D
            den = _rnd(jnp.sqrt(_rnd(_rnd(var) + LN_EPS)))
            xn = _rnd(_rnd(x - _rnd(mean)) * (1.0 / den))
            set_act(A_XN, t0, xn)
            if packed:
                act_buf[pl.ds(pl.multiple_of(A_XB + t0 // 2, 8), n // 2), :] = _pack(xn)

        def layernorm_pieces(t0):
            for p in range(4):
                layernorm(pl.multiple_of(t0 + p * (LNB // 2), LNB // 2), LNB // 2, False)
                yield

        def gate_pieces(blk):
            wr = wr_buf[...].astype(F32).reshape(1, D)
            best = None
            for p in range(LNB // LNP):
                t0 = pl.multiple_of(blk * LNB + p * LNP, LNP)
                xn = act(A_XN, t0, LNP)
                set_act(A_G, t0, _rnd(_silu_bounded(xn)))
                r = _rnd(jnp.sum(xn * wr, axis=1, keepdims=True))
                r = jnp.broadcast_to(r, (LNP, 128))
                bits = lax.shift_right_logical(pltpu.bitcast(r, I32), 16)
                rank = jnp.where(r < 0, 0xFFFF - bits, (bits & 0x7FFF) + 0x8000)
                rank = jnp.where(r != r, 0, rank)
                row = lax.broadcasted_iota(I32, (LNP, 128), 0) + p * LNP
                lane = lax.broadcasted_iota(I32, (LNP, 128), 1)
                key = KEY_BIAS + rank * S + (S - 1 - blk * LNB - lane)
                key = pltpu.bitcast(jnp.where(row == lane, key, 0), F32)
                best = key if best is None else jnp.maximum(best, key)
                yield
            key_buf[pl.ds(blk, 1), :] = jnp.max(best, axis=0, keepdims=True)

        def unzip_pieces(u):
            for t in (0, 2):
                for r in range(0, D // 2, D // 4):
                    rows = pl.ds(r, D // 4)
                    a = w_buf[4 * u + t, rows, :]
                    b = w_buf[4 * u + t + 1, rows, :]
                    w_buf[4 * u + t, rows, :] = (a & np.uint32(0xFFFF)) | (b << 16)
                    w_buf[4 * u + t + 1, rows, :] = (a >> 16) | (b & np.uint32(0xFFFF0000))
                    yield

        def project_pieces(j, m, odd):
            r0 = 0
            for n in PRO_BLOCKS:
                w = _cat([w_buf[4 * (3 * j + m) + t] for t in range(4)], 1)
                y = _nn(_as_bf(act_buf[pl.ds(A_XB + r0, n // 2), :]), _as_bf(w))
                qkv_bufs[2 * m + odd].at[j // 2][pl.ds(2 * r0, n), :] = y.astype(BF)
                r0 += n // 2
                yield

        cp_x0.wait()
        cp_wr.wait()
        start_weights(0)

        def first_ln(i, carry):
            layernorm(pl.multiple_of(i * (LN0 // 3), LN0 // 3), LN0 // 3, True)
            return carry

        lax.fori_loop(0, 3, first_ln, 0)
        for cp in weight_copies(0, 0):
            cp.wait()
        _interleave(unzip_pieces(0))

        def two_quads(i, carry):
            for odd in range(2):
                j = 2 * i + odd
                for jm in ((j, 1), (j, 2), (j + 1, 0)):
                    for cp in weight_copies(*jm):
                        cp.wait()
                if odd:
                    pl.when(i == 0)(cp_x1.wait)
                    pl.when(i < H // 8 - 1)(functools.partial(start_weights, j + 1))
                    for k, cp in enumerate((cp_wo, cp_wu, cp_mem)):
                        pl.when(i == k)(cp.start)
                else:
                    start_weights(j + 1)
                    for k, cp in enumerate((cp_x1, cp_wg, cp_wd)):
                        pl.when(i == k)(cp.start)
                t0 = jnp.clip(LN0 + (j - 1) * 2 * LNB, LN0 - 2 * LNB, TOK - 2 * LNB)
                for m in range(3):
                    side = gate_pieces(2 * j + m) if m < 2 else layernorm_pieces(t0)
                    _interleave(project_pieces(j, m, odd), unzip_pieces(3 * j + m + 1), side)
            return carry

        lax.fori_loop(0, H // 8, two_quads, 0)

        keys = key_buf[...]
        crow = lax.broadcasted_iota(I32, (C, 128), 0)
        top = jnp.zeros((C, 128), I32)
        idxs = []
        for c in range(C):
            kmax = jnp.max(jnp.max(keys, axis=0, keepdims=True), axis=1, keepdims=True)
            keys = jnp.where(keys == kmax, 0.0, keys)
            kbits = pltpu.bitcast(jnp.broadcast_to(kmax, (C, 128)), I32)
            top = jnp.where(crow == c, kbits, top)
            idx = jnp.max((S - 1 - (kbits & (S - 1))).astype(F32)).astype(I32)
            idx = jnp.clip(idx, 0, S - 1)
            idxs.append(idx)
            sel_buf[pl.ds(c, 1), :] = act_buf[pl.ds(A_XN + idx, 1), :]
        rank = lax.shift_right_logical(top - KEY_BIAS, 11)
        rbits = jnp.where(rank >= 0x8000, rank - 0x8000, 0xFFFF - rank)
        r_sel = pltpu.bitcast(rbits << 16, F32)[:, 0:1]
        cp_wg.wait()
        cp_wu.wait()
        cp_wd.wait()
        xs = pltpu.bitcast(sel_buf[...], F32)
        gate = _rnd(_silu(_rnd(_nt(xs, wg_buf[...]))))
        up = _rnd(_nt(xs, wu_buf[...]))
        y = _rnd(_nn(_rnd(gate * up), wd_buf[...]))
        y = _rnd(y * _rnd(jax.nn.sigmoid(r_sel)))
        g_sel = pltpu.bitcast(_rnd(_silu(_rnd(xs + y))), U32)
        for c in range(C):
            act_buf[pl.ds(A_G + idxs[c], 1), :] = g_sel[c:c + 1]
        cp_wo.wait()
        cp_mem.wait()

    if not ONLY_MAIN: pl.run_scoped(
        prologue,
        pltpu.VMEM((D,), BF),
        pltpu.VMEM((FF, D), BF),
        pltpu.VMEM((FF, D), BF),
        pltpu.VMEM((FF, D), BF),
        pltpu.VMEM((S // LNB, 128), F32),
        pltpu.VMEM((C, D), U32),
        pltpu.SemaphoreType.DMA((8,)),
        pltpu.SemaphoreType.DMA((3 * (H // 4) + 1,)),
    )

    def scan(out_buf, sems, o_raw, px_raw, pm_buf, km_raw, vm_raw, om_raw):
        o_buf, px_buf, km_buf, vm_buf, om_buf = (
            r.bitcast(BF) for r in (o_raw, px_raw, km_raw, vm_raw, om_raw))
        o_buf[:, pl.ds(0, FRONT), :] = jnp.zeros((H // 4, FRONT, 4 * E), BF)
        nk = SEG + 16
        row = lax.broadcasted_iota(I32, (M + SEG, nk), 0) - M
        col = lax.broadcasted_iota(I32, (M + SEG, nk), 1)
        visible = ((col <= row) | (row < 0) | (col >= SEG)) & (col < SEG + M)
        fill = jnp.where(col < SEG + M, -1e9 * LOG2E, -jnp.inf).astype(F32)
        zeros = jnp.zeros((M, 4 * E), F32)

        def softmax(s, r0, r1):
            s = jnp.where(visible[r0:r1], s * (E ** -0.5 * LOG2E), fill[r0:r1])
            e = jnp.exp2(s - jnp.max(s, axis=1, keepdims=True))
            return e * _recip(jnp.sum(e, axis=1, keepdims=True))

        def finish(r, n, s):
            x = x_buf[pl.ds(r, n), :].astype(F32)
            out_buf[pl.ds(r, n), :] = (x + _rnd(_rnd(s) * act(A_G - FRONT, r, n))).astype(BF)

        def step(s, par, mem):
            seg = pl.multiple_of(s * SEG, SEG)
            rin = pl.multiple_of(PRO + RIDE * s, 8)
            rout = pl.multiple_of(RIDE * s + FRONT - RIDE, 8)
            win = pl.multiple_of(rin - 8 * par, 16)
            wout = pl.multiple_of(rout - 8 * (1 - par), 16)
            lhs = _cat([mem, act(A_XN, rin, RIDE)]).astype(BF)
            qm, om, acc = {}, {}, []

            def seg_rows(m, h):
                j, t = divmod(h, 4)
                return qkv_bufs[2 * m + j % 2][j // 2, pl.ds(seg, SEG), t * E:(t + 1) * E]

            def project(jm):
                j, m = jm
                w = _as_bf(_cat([w_buf[4 * (3 * j + m) + t] for t in range(4)], 1))
                y = None
                for k in range(0, D, E):
                    z = _nn(lhs[:, k:k + E], w[k:k + E])
                    y = z if y is None else y + z
                dst = qkv_bufs[2 * m + j % 2].at[j // 2, pl.ds(win, 32), :]
                if par == 0:
                    dst[0:16, :] = y[8:24].astype(BF)
                    dst[16:24, :] = y[24:32].astype(BF)
                else:
                    dst[8:16, :] = y[8:16].astype(BF) if not HALF else y[0:16].astype(BF)[8:16]
                    dst[16:32, :] = y[16:32].astype(BF)
                if m == 0:
                    qm[j] = _rnd(y[0:M])
                else:
                    (km_buf if m == 1 else vm_buf).at[j][...] = _cat([y[0:M], zeros]).astype(BF)

            def with_mem(m, h):
                j, t = divmod(h, 4)
                return _cat([seg_rows(m, h), (km_buf if m == 1 else vm_buf)[j, :, t * E:(t + 1) * E]])

            def q_mem(h):
                return qm[h // 4][:, (h % 4) * E:(h % 4 + 1) * E]

            def px_at(h):
                return px_buf.at[h // 4, :, pl.ds((h % 4) * E, nk)]

            def qk_m(h):
                pm_buf[h, 0:M] = _rnd(softmax(_nt(q_mem(h), with_mem(1, h)), 0, M))

            def qk_x(h):
                px_at(h)[...] = softmax(_nt(seg_rows(0, h), with_mem(1, h)), M, M + SEG).astype(BF)

            def qk_all(h):
                q = _cat([q_mem(h), seg_rows(0, h).astype(F32)])
                p = softmax(_nt(q, with_mem(1, h)), 0, M + SEG)
                if h < H - TAILX and MERGE_PV:
                    pm_buf[h] = _rnd(p)
                else:
                    pm_buf[h, 0:M] = _rnd(p[0:M])
                    px_at(h)[...] = p[M:].astype(BF)

            def put_o(h, o):
                o_buf.at[h // 4][pl.ds(seg + FRONT, SEG), (h % 4) * E:(h % 4 + 1) * E] = o.astype(BF)

            def pv_m(h):
                om[h] = _nn(pm_buf[h, 0:M], with_mem(2, h))

            def pv_x(h):
                put_o(h, _nn(px_at(h)[...], with_mem(2, h)))

            def pv_all(h):
                o = _nn(pm_buf[h], with_mem(2, h))
                om[h] = o[0:M]
                put_o(h, o[M:])

            def out_proj(h):
                j, t = divmod(h, 4)
                lanes = slice(t * E, (t + 1) * E)
                lo = o_buf[j, pl.ds(wout, 16), lanes]
                hi = o_buf[j, pl.ds(wout + 16, 16), lanes]
                full, half = (hi, lo.astype(F32)[8:16]) if par == 0 else (lo, hi.astype(F32)[0:8])
                om_buf.at[j][:, lanes] = _cat([om[h], half]).astype(BF)
                y = _nn(_cat([om_buf[j, :, lanes], full]), _as_bf(wo_buf[h]))
                acc[:] = [y if not acc else acc[0] + y]

            order = [(3 * j + m, 0, project, (j, m)) for j in range(H // 4) for m in range(3)]
            order += [(24 + h / 4, 0, out_proj, h) for h in range(H)]
            for h in range(H):
                j = h // 4
                if MERGE_QK:
                    order.append((3 * j + LQ - 0.5, OQ, qk_all, h))
                else:
                    order.append((3 * j + LQM - 0.5, OQM, qk_m, h))
                    order.append((3 * j + LQ - 0.5, OQ, qk_x, h))
                if h < H - TAILX and MERGE_PV:
                    order.append((3 * j + LP - 0.5, OP, pv_all, h))
                else:
                    order.append((3 * j + LPM - 0.5, OPM, pv_m, h))
                    order.append((3 * j + LP - 0.5 if h < H - TAILX else 1000, OP, pv_x, h))
            order.sort(key=lambda e: e[:2])
            for _, _, fn, arg in order:
                fn(arg)

            y = acc[0]
            finish(rout, RIDE, y[8:32] if par == 0 else _cat([y[16:32], y[8:16]]))
            return _rnd(y[0:M])

        def steps(i, mem):
            for k in range(UNROLL):
                mem = step(UNROLL * i + k, k % 2, mem)
            return mem

        lax.fori_loop(0, NSEG // UNROLL, steps, mem_buf[...].astype(F32))

        copies = [pltpu.make_async_copy(out_buf.at[pl.ds(FRONT, EPI0)], out_hbm.at[pl.ds(0, EPI0)],
                                        sems.at[0])]
        copies[0].start()
        t = EPI0
        for b, n in enumerate((144, 144, 128, 128) if not ONLY_MAIN else ()):
            o = _cat([o_buf[j, pl.ds(FRONT + t, n), :] for j in range(H // 4)], 1)
            w = _as_bf(wo_buf[...].reshape(H * E // 2, D))
            finish(FRONT + t, n, _nn(o, w))
            copies.append(pltpu.make_async_copy(out_buf.at[pl.ds(FRONT + t, n)],
                                                out_hbm.at[pl.ds(t, n)], sems.at[1 + b]))
            copies[-1].start()
            t += n
        for cp in copies:
            cp.wait()

    pl.run_scoped(
        scan,
        pltpu.VMEM((FRONT + S, D), BF),
        pltpu.SemaphoreType.DMA((5,)),
        pltpu.VMEM((H // 4, (FRONT + S) // 2, 4 * E), U32),
        pltpu.VMEM((H // 4, SEG // 2, 4 * E), U32),
        pltpu.VMEM((H, M + SEG, SEG + 16), F32),
        *[pltpu.VMEM((H // 4, 8, 4 * E), U32) for _ in range(3)],
    )


@functools.partial(jax.jit, static_argnames=("A_seg_len",))
def pallas_recurrent_scan__memory_aug_recurrent_mem_tr__moe_arch_mod__prompt_kernel(
    A_x: jax.Array,
    A_mem0: jax.Array,
    A_Wq: jax.Array,
    A_Wk: jax.Array,
    A_Wv: jax.Array,
    A_Wo: jax.Array,
    A_seg_len: int,
    B_x: jax.Array,
    B_w_r: jax.Array,
    B_w_gate: jax.Array,
    B_w_up: jax.Array,
    B_w_down: jax.Array,
):
    del B_x
    assert A_seg_len == SEG and A_x.shape == (1, S, D) and A_mem0.shape == (1, M, D)
    assert A_Wq.shape == (D, H, E) and A_Wo.shape == (H, E, D) and B_w_gate.shape == (D, FF)
    hbm = pl.BlockSpec(memory_space=pltpu.MemorySpace.HBM)
    out = pl.pallas_call(
        _kernel,
        out_shape=jax.ShapeDtypeStruct((S, D), BF),
        in_specs=[hbm] * 10,
        out_specs=hbm,
        scratch_shapes=[
            pltpu.VMEM((FRONT + TOK, D), BF),
            pltpu.VMEM((A_XB + LN0 // 2, D), U32),
            pltpu.VMEM((H, E // 2, D), U32),
            pltpu.VMEM((M, D), BF),
            pltpu.VMEM((3 * H + 4, D // 2, E), U32),
            *[pltpu.VMEM((H // 8, QROWS // 2, 4 * E), U32) for _ in range(6)],
        ],
        compiler_params=pltpu.CompilerParams(vmem_limit_bytes=124 * 1024 * 1024),
    )(A_x.reshape(S, D), A_mem0.reshape(M, D),
      *(w.reshape(D // 2, 2, H, E) for w in (A_Wq, A_Wk, A_Wv)), A_Wo, B_w_r, B_w_gate.T, B_w_up.T,
      B_w_down)
    return out.reshape(1, S, D)
```

```python
import functools

import jax
import jax.numpy as jnp
import numpy as np
from jax import lax
import jax.experimental.pallas as pl
import jax.experimental.pallas.tpu as pltpu

BF = jnp.bfloat16
F32 = jnp.float32
U32 = jnp.uint32
I32 = jnp.int32

S, D, H, E, M, SEG, FF, C = 2048, 640, 32, 128, 8, 32, 1728, 8
NSEG = S // SEG
NQ = H // 4
RIDE = 24
PRO_BLOCKS = (144, 144, 128, 128)
PRO = sum(PRO_BLOCKS)
EPI_BLOCKS = (144, 144, 128, 128)
EPI0 = S - sum(EPI_BLOCKS)
FRONT = 32
QROWS = PRO + RIDE * NSEG
LN0 = 576
LNJ = 256
TOK = LN0 + 6 * LNJ
A_XN, A_G, A_XB = 0, TOK + FRONT, TOK + FRONT + S
NK = SEG + 16
UNROLL = 4
TAIL = 12
KEY_BIAS = 0x10000000
LN_EPS = 1.0013580322265625e-05
LOG2E = 1.4426950408889634


def _nn(a, b):
    return lax.dot_general(a, b, (((1,), (0,)), ((), ())), preferred_element_type=F32)


def _nt(a, b):
    return lax.dot_general(a, b, (((1,), (1,)), ((), ())), preferred_element_type=F32)


def _as_bf(x):
    return pltpu.bitcast(x, BF)


def _rnd(x):
    return x.astype(BF).astype(F32)


def _cat(xs, axis=0):
    return jnp.concatenate(xs, axis)


def _recip(x):
    r = pl.reciprocal(x, approx=True)
    return r * (2.0 - x * r)


def _silu(x):
    return x * jax.nn.sigmoid(x)


def _interleave(*gens):
    gens = list(gens)
    while gens:
        gens = [g for g in gens if next(g, StopIteration) is not StopIteration]


def _kernel(x_hbm, mem_hbm, wq_hbm, wk_hbm, wv_hbm, wo_hbm, wr_hbm, wg_hbm, wu_hbm, wd_hbm,
            out_hbm, x_buf, act_buf, wo_buf, mem_buf, w_buf, *qkv_raw):
    qkv = [r.bitcast(BF) for r in qkv_raw]

    def act(base, r, n):
        return pltpu.bitcast(act_buf[pl.ds(base + r, n), :], F32)

    def set_act(base, r, val):
        act_buf[pl.ds(base + r, val.shape[0]), :] = pltpu.bitcast(val, U32)

    def quad_weight(j, m):
        return _as_bf(_cat([w_buf[4 * (3 * j + m) + t] for t in range(4)], 1))

    def prologue(wr_buf, wg_buf, wu_buf, wd_buf, key_buf, sel_buf, sems, wsems):
        srcs = [w.bitcast(U32) for w in (wq_hbm, wk_hbm, wv_hbm)]
        copy = pltpu.make_async_copy
        cp_x0 = copy(x_hbm.at[pl.ds(0, LN0)], x_buf.at[pl.ds(FRONT, LN0)], sems.at[0])
        cp_x1 = copy(x_hbm.at[pl.ds(LN0, S - LN0)], x_buf.at[pl.ds(FRONT + LN0, S - LN0)],
                     sems.at[1])
        cp_wr = copy(wr_hbm, wr_buf, sems.at[2])
        cp_mem = copy(mem_hbm, mem_buf, sems.at[3])
        cp_wo = copy(wo_hbm.bitcast(U32), wo_buf, sems.at[4])
        cp_wg = copy(wg_hbm, wg_buf, sems.at[5])
        cp_wu = copy(wu_hbm, wu_buf, sems.at[6])
        cp_wd = copy(wd_hbm, wd_buf, sems.at[7])

        def weight_copies(*units):
            return [copy(srcs[m].at[:, t % 2, 2 * jnp.minimum(j, NQ - 1) + t // 2, :],
                         w_buf.at[4 * (3 * j + m) + t], wsems.at[3 * j + m])
                    for j, m in units for t in range(4)]

        def next_weights(j):
            return weight_copies((j, 1), (j, 2), (j + 1, 0))

        def start(copies):
            for cp in copies:
                cp.start()

        def wait(copies):
            for cp in copies:
                cp.wait()

        def unzip(u):
            for t in (0, 2):
                for r in (0, D // 4):
                    rows = pl.ds(r, D // 4)
                    a = w_buf[4 * u + t, rows, :]
                    b = w_buf[4 * u + t + 1, rows, :]
                    w_buf[4 * u + t, rows, :] = (a & np.uint32(0xFFFF)) | (b << 16)
                    w_buf[4 * u + t + 1, rows, :] = (a >> 16) | (b & np.uint32(0xFFFF0000))
                    yield

        def layernorm(t0, n):
            x = x_buf[pl.ds(FRONT + t0, n), :].astype(F32)
            mean = jnp.sum(x, axis=1, keepdims=True) / D
            cen = x - mean
            var = jnp.sum(cen * cen, axis=1, keepdims=True) / D
            den = _rnd(jnp.sqrt(_rnd(_rnd(var) + LN_EPS)))
            xn = _rnd(_rnd(x - _rnd(mean)) * (1.0 / den))
            set_act(A_XN, t0, xn)
            return xn

        def layernorm_pieces(t0):
            for p in range(4):
                layernorm(pl.multiple_of(t0 + p * (LNJ // 4), LNJ // 4), LNJ // 4)
                yield

        def gate_pieces(blk):
            wr = wr_buf[...].astype(F32).reshape(1, D)
            best = None
            for p in range(0, 128, 32):
                t0 = pl.multiple_of(blk * 128 + p, 32)
                xn = act(A_XN, t0, 32)
                set_act(A_G, t0, _rnd(xn * _recip(1.0 + jnp.exp(-xn))))
                r = jnp.broadcast_to(_rnd(jnp.sum(xn * wr, axis=1, keepdims=True)), (32, 128))
                bits = lax.shift_right_logical(pltpu.bitcast(r, I32), 16)
                rank = jnp.where(r < 0, 0xFFFF - bits, (bits & 0x7FFF) + 0x8000)
                rank = jnp.where(r != r, 0, rank)
                row = lax.broadcasted_iota(I32, (32, 128), 0) + p
                lane = lax.broadcasted_iota(I32, (32, 128), 1)
                key = KEY_BIAS + rank * S + (S - 1 - blk * 128 - lane)
                key = pltpu.bitcast(jnp.where(row == lane, key, 0), F32)
                best = key if best is None else jnp.maximum(best, key)
                yield
            key_buf[pl.ds(blk, 1), :] = jnp.max(best, axis=0, keepdims=True)

        def project_pieces(j, m, odd):
            r = 0
            for n in PRO_BLOCKS:
                y = _nn(_as_bf(act_buf[pl.ds(A_XB + r // 2, n // 2), :]), quad_weight(j, m))
                qkv[2 * m + odd].at[j // 2][pl.ds(r, n), :] = y.astype(BF)
                r += n
                yield

        start([cp_x0, cp_wr, *weight_copies((0, 0))])
        x_buf[pl.ds(0, FRONT), :] = jnp.zeros((FRONT, D), BF)
        x_buf[pl.ds(FRONT + S, TOK - S), :] = jnp.zeros((TOK - S, D), BF)
        set_act(A_G - FRONT, 0, jnp.zeros((FRONT, D), F32))
        wait([cp_x0, cp_wr])
        start(next_weights(0))

        def first_layernorm(i, carry):
            n = LN0 // 3
            xn = layernorm(pl.multiple_of(i * n, n), n)
            act_buf[pl.ds(pl.multiple_of(A_XB + i * (n // 2), 8), n // 2), :] = pltpu.bitcast(
                xn.astype(BF), U32)
            return carry

        lax.fori_loop(0, 3, first_layernorm, 0)
        wait(weight_copies((0, 0)))
        _interleave(unzip(0))

        def two_quads(i, carry):
            for odd in range(2):
                j = 2 * i + odd
                wait(next_weights(j))
                if odd:
                    pl.when(i == 0)(cp_x1.wait)
                    pl.when(j < NQ - 1)(lambda: start(next_weights(j + 1)))
                else:
                    start(next_weights(j + 1))
                for k, cp in enumerate((cp_wo, cp_wu, cp_mem) if odd else (cp_x1, cp_wg, cp_wd)):
                    pl.when(i == k)(cp.start)
                t0 = jnp.clip(LN0 + (j - 1) * LNJ, LN0 - LNJ, TOK - LNJ)
                for m in range(3):
                    _interleave(project_pieces(j, m, odd), unzip(3 * j + m + 1),
                                gate_pieces(2 * j + m) if m < 2 else layernorm_pieces(t0))
            return carry

        lax.fori_loop(0, NQ // 2, two_quads, 0)

        keys = key_buf[...]
        crow = lax.broadcasted_iota(I32, (C, 128), 0)
        top = jnp.zeros((C, 128), I32)
        idxs = []
        for c in range(C):
            kmax = jnp.max(jnp.max(keys, axis=0, keepdims=True), axis=1, keepdims=True)
            keys = jnp.where(keys == kmax, 0.0, keys)
            kbits = pltpu.bitcast(jnp.broadcast_to(kmax, (C, 128)), I32)
            top = jnp.where(crow == c, kbits, top)
            idx = jnp.max((S - 1 - (kbits & (S - 1))).astype(F32)).astype(I32)
            idxs.append(jnp.clip(idx, 0, S - 1))
            sel_buf[pl.ds(c, 1), :] = act_buf[pl.ds(A_XN + idxs[c], 1), :]
        rank = lax.shift_right_logical(top - KEY_BIAS, 11)
        rbits = jnp.where(rank >= 0x8000, rank - 0x8000, 0xFFFF - rank)
        r_sel = pltpu.bitcast(rbits << 16, F32)[:, 0:1]
        wait([cp_wg, cp_wu, cp_wd])
        xs = pltpu.bitcast(sel_buf[...], F32)
        gate = _rnd(_silu(_rnd(_nt(xs, wg_buf[...]))))
        up = _rnd(_nt(xs, wu_buf[...]))
        y = _rnd(_nn(_rnd(gate * up), wd_buf[...]))
        y = _rnd(y * _rnd(jax.nn.sigmoid(r_sel)))
        g_sel = pltpu.bitcast(_rnd(_silu(_rnd(xs + y))), U32)
        for c in range(C):
            act_buf[pl.ds(A_G + idxs[c], 1), :] = g_sel[c:c + 1]
        wait([cp_wo, cp_mem])

    def scan(out_buf, sems, pm_buf, *raw):
        o_buf, px_buf, km_buf, vm_buf, om_buf = (r.bitcast(BF) for r in raw)
        o_buf[:, pl.ds(0, FRONT), :] = jnp.zeros((NQ, FRONT, 4 * E), BF)
        row = lax.broadcasted_iota(I32, (M + SEG, NK), 0) - M
        col = lax.broadcasted_iota(I32, (M + SEG, NK), 1)
        visible = ((col <= row) | (row < 0) | (col >= SEG)) & (col < SEG + M)
        fill = jnp.where(col < SEG + M, -1e9 * LOG2E, -jnp.inf).astype(F32)
        zeros = jnp.zeros((M, 4 * E), F32)

        def finish(r, n, s):
            x = x_buf[pl.ds(r, n), :].astype(F32)
            out_buf[pl.ds(r, n), :] = (x + _rnd(_rnd(s) * act(A_G - FRONT, r, n))).astype(BF)

        def step(s, odd, mem):
            seg = pl.multiple_of(s * SEG, SEG)
            rin = pl.multiple_of(PRO + RIDE * s, 8)
            rout = pl.multiple_of(RIDE * (s - 1) + FRONT, 8)
            win = pl.multiple_of(rin - 8 * odd, 16)
            wout = pl.multiple_of(rout - 8 * (1 - odd), 16)
            lhs = _cat([mem, act(A_XN, rin, RIDE)]).astype(BF)
            qm, om, acc = {}, {}, []

            def lanes(h):
                return slice(h % 4 * E, (h % 4 + 1) * E)

            def seg_rows(m, h):
                j = h // 4
                return qkv[2 * m + j % 2][j // 2, pl.ds(seg, SEG), lanes(h)]

            def with_mem(m, h):
                return _cat([seg_rows(m, h), (km_buf if m == 1 else vm_buf)[h // 4, :, lanes(h)]])

            def px(h):
                return px_buf.at[h // 4, :, pl.ds(h % 4 * E, NK)]

            def put_o(h, o):
                o_buf.at[h // 4][pl.ds(seg + FRONT, SEG), lanes(h)] = o.astype(BF)

            def project(j, m):
                w = quad_weight(j, m)
                y = _nn(lhs[:, 0:E], w[0:E])
                for k in range(E, D, E):
                    y += _nn(lhs[:, k:k + E], w[k:k + E])
                dst = qkv[2 * m + j % 2].at[j // 2, pl.ds(win, 32), :]
                if odd:
                    dst[8:16, :] = y[8:16].astype(BF)
                    dst[16:32, :] = y[16:32].astype(BF)
                else:
                    dst[0:16, :] = y[8:24].astype(BF)
                    dst[16:24, :] = y[24:32].astype(BF)
                if m == 0:
                    qm[j] = _rnd(y[0:M])
                else:
                    (km_buf if m == 1 else vm_buf).at[j][...] = _cat([y[0:M], zeros]).astype(BF)

            def scores(h):
                q = _cat([qm[h // 4][:, lanes(h)], seg_rows(0, h).astype(F32)])
                sc = jnp.where(visible, _nt(q, with_mem(1, h)) * (E ** -0.5 * LOG2E), fill)
                e = jnp.exp2(sc - jnp.max(sc, axis=1, keepdims=True))
                p = e * _recip(jnp.sum(e, axis=1, keepdims=True))
                if h < H - TAIL:
                    pm_buf[h] = _rnd(p)
                else:
                    pm_buf[h, 0:M] = _rnd(p[0:M])
                    px(h)[...] = p[M:].astype(BF)

            def mix(h):
                o = _nn(pm_buf[h], with_mem(2, h))
                om[h] = o[0:M]
                put_o(h, o[M:])

            def mix_mem(h):
                om[h] = _nn(pm_buf[h, 0:M], with_mem(2, h))

            def mix_seg(h):
                put_o(h, _nn(px(h)[...], with_mem(2, h)))

            def out_proj(h):
                lo = o_buf[h // 4, pl.ds(wout, 16), lanes(h)]
                hi = o_buf[h // 4, pl.ds(wout + 16, 16), lanes(h)]
                full, half = (lo, hi.astype(F32)[0:8]) if odd else (hi, lo.astype(F32)[8:16])
                om_buf.at[h // 4][:, lanes(h)] = _cat([om[h], half]).astype(BF)
                y = _nn(_cat([om_buf[h // 4, :, lanes(h)], full]), _as_bf(wo_buf[h]))
                acc[:] = [acc[0] + y if acc else y]

            order = [(3 * j + m, project, j, m) for j in range(NQ) for m in range(3)]
            order += [(3 * NQ + h / 4, out_proj, h) for h in range(H)]
            for h in range(H):
                t = 3 * (h // 4)
                order.append((t + 3.5, scores, h))
                if h < H - TAIL:
                    order.append((t + 7.5, mix, h))
                else:
                    order += [(t + 6.4, mix_mem, h), (4 * NQ, mix_seg, h)]
            for _, fn, *args in sorted(order, key=lambda e: e[0]):
                fn(*args)

            y = acc[0]
            finish(rout, RIDE, _cat([y[16:32], y[8:16]]) if odd else y[8:32])
            return _rnd(y[0:M])

        def steps(i, mem):
            for k in range(UNROLL):
                mem = step(UNROLL * i + k, k % 2, mem)
            return mem

        lax.fori_loop(0, NSEG // UNROLL, steps, mem_buf[...].astype(F32))

        def write_out(t, n, k):
            cp = pltpu.make_async_copy(out_buf.at[pl.ds(FRONT + t, n)], out_hbm.at[pl.ds(t, n)],
                                       sems.at[k])
            cp.start()
            return cp

        copies = [write_out(0, EPI0, 0)]
        t = EPI0
        for n in EPI_BLOCKS:
            o = _cat([o_buf[j, pl.ds(FRONT + t, n), :] for j in range(NQ)], 1)
            finish(FRONT + t, n, _nn(o, _as_bf(wo_buf[...].reshape(H * E // 2, D))))
            copies.append(write_out(t, n, len(copies)))
            t += n
        for cp in copies:
            cp.wait()

    pl.run_scoped(
        prologue,
        pltpu.VMEM((D,), BF),
        *[pltpu.VMEM((FF, D), BF) for _ in range(3)],
        pltpu.VMEM((S // 128, 128), F32),
        pltpu.VMEM((C, D), U32),
        pltpu.SemaphoreType.DMA((8,)),
        pltpu.SemaphoreType.DMA((3 * NQ + 1,)),
    )
    pl.run_scoped(
        scan,
        pltpu.VMEM((FRONT + S, D), BF),
        pltpu.SemaphoreType.DMA((1 + len(EPI_BLOCKS),)),
        pltpu.VMEM((H, M + SEG, NK), F32),
        pltpu.VMEM((NQ, (FRONT + S) // 2, 4 * E), U32),
        pltpu.VMEM((NQ, SEG // 2, 4 * E), U32),
        *[pltpu.VMEM((NQ, 8, 4 * E), U32) for _ in range(3)],
    )


@functools.partial(jax.jit, static_argnames=("A_seg_len",))
def pallas_recurrent_scan__memory_aug_recurrent_mem_tr__moe_arch_mod__prompt_kernel(
    A_x: jax.Array,
    A_mem0: jax.Array,
    A_Wq: jax.Array,
    A_Wk: jax.Array,
    A_Wv: jax.Array,
    A_Wo: jax.Array,
    A_seg_len: int,
    B_x: jax.Array,
    B_w_r: jax.Array,
    B_w_gate: jax.Array,
    B_w_up: jax.Array,
    B_w_down: jax.Array,
):
    del B_x
    assert A_seg_len == SEG and A_x.shape == (1, S, D) and A_mem0.shape == (1, M, D)
    assert A_Wq.shape == (D, H, E) and A_Wo.shape == (H, E, D) and B_w_gate.shape == (D, FF)
    hbm = pl.BlockSpec(memory_space=pltpu.MemorySpace.HBM)
    out = pl.pallas_call(
        _kernel,
        out_shape=jax.ShapeDtypeStruct((S, D), BF),
        in_specs=[hbm] * 10,
        out_specs=hbm,
        scratch_shapes=[
            pltpu.VMEM((FRONT + TOK, D), BF),
            pltpu.VMEM((A_XB + LN0 // 2, D), U32),
            pltpu.VMEM((H, E // 2, D), U32),
            pltpu.VMEM((M, D), BF),
            pltpu.VMEM((3 * H + 4, D // 2, E), U32),
            *[pltpu.VMEM((NQ // 2, QROWS // 2, 4 * E), U32) for _ in range(6)],
        ],
        compiler_params=pltpu.CompilerParams(vmem_limit_bytes=124 * 1024 * 1024),
    )(A_x.reshape(S, D), A_mem0.reshape(M, D),
      *(w.reshape(D // 2, 2, H, E) for w in (A_Wq, A_Wk, A_Wv)), A_Wo,
      B_w_r, B_w_gate.T, B_w_up.T, B_w_down)
    return out.reshape(1, S, D)
```

```python
import functools

import jax
import jax.numpy as jnp
import numpy as np
from jax import lax
import jax.experimental.pallas as pl
import jax.experimental.pallas.tpu as pltpu

BF = jnp.bfloat16
F32 = jnp.float32
U32 = jnp.uint32
I32 = jnp.int32

S, D, H, E, M, SEG, FF, C = 2048, 640, 32, 128, 8, 32, 1728, 8
NSEG = S // SEG
NQ = H // 4
RIDE = 24
PRO_BLOCKS = (144, 128, 128, 128)
PRO = sum(PRO_BLOCKS)
EPI_BLOCKS = (192, 192, 128, 48)
EPI0 = S - sum(EPI_BLOCKS)
FRONT = 32
QROWS = PRO + RIDE * NSEG
LN0 = PRO
LNJ = 256
TOK = LN0 + 6 * LNJ
A_XN, A_G, A_XB = 0, TOK + FRONT, TOK + FRONT + S
NK = SEG + 16
UNROLL = 4
TAIL = 10
KEY_BIAS = 0x10000000
LN_EPS = 1.0013580322265625e-05
LOG2E = 1.4426950408889634


def _nn(a, b):
    return lax.dot_general(a, b, (((1,), (0,)), ((), ())), preferred_element_type=F32)


def _nt(a, b):
    return lax.dot_general(a, b, (((1,), (1,)), ((), ())), preferred_element_type=F32)


def _as_bf(x):
    return pltpu.bitcast(x, BF)


def _rnd(x):
    return x.astype(BF).astype(F32)


def _cat(xs, axis=0):
    return jnp.concatenate(xs, axis)


def _recip(x):
    r = pl.reciprocal(x, approx=True)
    return r * (2.0 - x * r)


def _silu(x):
    return x * jax.nn.sigmoid(x)


def _aligned(x, n):
    return x if isinstance(x, int) else pl.multiple_of(x, n)


def _interleave(*gens):
    gens = list(gens)
    while gens:
        gens = [g for g in gens if next(g, StopIteration) is not StopIteration]


def _kernel(x_hbm, mem_hbm, wq_hbm, wk_hbm, wv_hbm, wo_hbm, wr_hbm, wg_hbm, wu_hbm, wd_hbm,
            out_hbm, x_buf, act_buf, wo_buf, mem_buf, w_buf, *qkv_raw):
    qkv = [r.bitcast(BF) for r in qkv_raw]

    def act(base, r, n):
        return pltpu.bitcast(act_buf[pl.ds(base + r, n), :], F32)

    def set_act(base, r, val):
        act_buf[pl.ds(base + r, val.shape[0]), :] = pltpu.bitcast(val, U32)

    def quad_weight(j, m):
        return _as_bf(_cat([w_buf[4 * (3 * j + m) + t] for t in range(4)], 1))

    def prologue(wr_buf, wg_buf, wu_buf, wd_buf, key_buf, sel_buf, sems, wsems):
        srcs = [w.bitcast(U32) for w in (wq_hbm, wk_hbm, wv_hbm)]
        copy = pltpu.make_async_copy
        cp_x0 = copy(x_hbm.at[pl.ds(0, LN0)], x_buf.at[pl.ds(FRONT, LN0)], sems.at[0])
        cp_x1 = copy(x_hbm.at[pl.ds(LN0, LNJ)], x_buf.at[pl.ds(FRONT + LN0, LNJ)], sems.at[1])
        cp_x2 = copy(x_hbm.at[pl.ds(LN0 + LNJ, S - LN0 - LNJ)],
                     x_buf.at[pl.ds(FRONT + LN0 + LNJ, S - LN0 - LNJ)], sems.at[8])
        cp_wr = copy(wr_hbm, wr_buf, sems.at[2])
        cp_mem = copy(mem_hbm, mem_buf, sems.at[3])
        cp_wo = copy(wo_hbm.bitcast(U32), wo_buf, sems.at[4])
        cp_wg = copy(wg_hbm, wg_buf, sems.at[5])
        cp_wu = copy(wu_hbm, wu_buf, sems.at[6])
        cp_wd = copy(wd_hbm, wd_buf, sems.at[7])

        def weight_copies(i, *units):
            return [copy(srcs[k % 3].at[:, t % 2, 2 * (2 * i + k // 3) + t // 2, :],
                         w_buf.at[4 * (6 * i + k) + t], wsems.at[6 * i + k])
                    for k in units for t in range(4)]

        def start(copies):
            for cp in copies:
                cp.start()

        def wait(copies):
            for cp in copies:
                cp.wait()

        def unzip(u):
            for t in (0, 2):
                for r in (0, D // 4):
                    rows = pl.ds(r, D // 4)
                    a = w_buf[4 * u + t, rows, :]
                    b = w_buf[4 * u + t + 1, rows, :]
                    w_buf[4 * u + t, rows, :] = (a & np.uint32(0xFFFF)) | (b << 16)
                    w_buf[4 * u + t + 1, rows, :] = (a >> 16) | (b & np.uint32(0xFFFF0000))
                    yield

        def layernorm(t0, n):
            x = x_buf[pl.ds(FRONT + t0, n), :].astype(F32)
            mean = jnp.sum(x, axis=1, keepdims=True) / D
            cen = x - mean
            var = jnp.sum(cen * cen, axis=1, keepdims=True) / D
            den = _rnd(jnp.sqrt(_rnd(_rnd(var) + LN_EPS)))
            xn = _rnd(_rnd(x - _rnd(mean)) * (1.0 / den))
            set_act(A_XN, t0, xn)
            return xn

        def layernorm_pieces(t0):
            for p in range(4):
                layernorm(pl.multiple_of(t0 + p * (LNJ // 4), 16), LNJ // 4)
                yield

        def gate_pieces(blk):
            wr = wr_buf[...].astype(F32).reshape(1, D)
            best = None
            for p in range(0, 128, 32):
                t0 = _aligned(blk * 128 + p, 32)
                xn = act(A_XN, t0, 32)
                set_act(A_G, t0, _rnd(xn * _recip(1.0 + jnp.exp(-xn))))
                r = jnp.broadcast_to(_rnd(jnp.sum(xn * wr, axis=1, keepdims=True)), (32, 128))
                bits = lax.shift_right_logical(pltpu.bitcast(r, I32), 16)
                rank = jnp.where(r < 0, 0xFFFF - bits, (bits & 0x7FFF) + 0x8000)
                rank = jnp.where(r != r, 0, rank)
                row = lax.broadcasted_iota(I32, (32, 128), 0) + p
                lane = lax.broadcasted_iota(I32, (32, 128), 1)
                key = KEY_BIAS + rank * S + (S - 1 - blk * 128 - lane)
                key = pltpu.bitcast(jnp.where(row == lane, key, 0), F32)
                best = key if best is None else jnp.maximum(best, key)
                yield
            key_buf[pl.ds(blk, 1), :] = jnp.max(best, axis=0, keepdims=True)

        def project_pieces(i, k):
            j, m, odd = 2 * i + k // 3, k % 3, k // 3 % 2
            r = 0
            for n in PRO_BLOCKS:
                y = _nn(_as_bf(act_buf[pl.ds(A_XB + r // 2, n // 2), :]), quad_weight(j, m))
                qkv[2 * m + odd].at[j // 2][pl.ds(r, n), :] = y.astype(BF)
                r += n
                yield

        start([cp_x0, cp_wr, *weight_copies(0, 0)])
        x_buf[pl.ds(0, FRONT), :] = jnp.zeros((FRONT, D), BF)
        x_buf[pl.ds(FRONT + S, TOK - S), :] = jnp.zeros((TOK - S, D), BF)
        set_act(A_G - FRONT, 0, jnp.zeros((FRONT, D), F32))
        wait([cp_x0, cp_wr])
        start(weight_copies(0, 1))

        def first_layernorm(i, carry):
            n = LN0 // 3
            xn = layernorm(pl.multiple_of(i * n, 16), n)
            act_buf[pl.ds(pl.multiple_of(A_XB + i * (n // 2), 8), n // 2), :] = pltpu.bitcast(
                xn.astype(BF), U32)
            pl.when(i == 0)(lambda: start([*weight_copies(0, 2, 3, 4), cp_x1]))
            return carry

        lax.fori_loop(0, 3, first_layernorm, 0)
        wait(weight_copies(0, 0, 1))
        _interleave(unzip(0))
        _interleave(project_pieces(0, 0), unzip(1))

        def six_units(i, carry):
            for half in range(2):
                k0 = 3 * half + 1
                wait(weight_copies(i, k0 + 1, k0 + 2, k0 + 3))
                pl.when(i == 0)((cp_x2 if half else cp_x1).wait)
                start(weight_copies(i, k0 + 4, k0 + 5, k0 + 6))
                for k, cp in enumerate((cp_wo, cp_wu, cp_mem) if half else (cp_x2, cp_wg, cp_wd)):
                    pl.when(i == k)(cp.start)
                blk = 4 * i + 2 * half
                sides = (gate_pieces(blk), gate_pieces(blk + 1),
                         layernorm_pieces(LN0 + (2 * i + half) * LNJ))
                for k, side in zip(range(k0, k0 + 3), sides):
                    _interleave(project_pieces(i, k), unzip(6 * i + k + 1), side)
            return blk + 2

        blk = lax.fori_loop(0, 3, six_units, 0)
        start(weight_copies(3, 5))
        wait(weight_copies(3, 2, 3, 4))
        for k in range(1, 4):
            _interleave(project_pieces(3, k), unzip(18 + k + 1), gate_pieces(blk + k - 1))
        wait([*weight_copies(3, 5), cp_wg, cp_wu, cp_wd, cp_wo, cp_mem])
        _interleave(project_pieces(3, 4), unzip(23), gate_pieces(blk + 3))
        _interleave(project_pieces(3, 5))

        keys = key_buf[...]
        crow = lax.broadcasted_iota(I32, (C, 128), 0)
        top = jnp.zeros((C, 128), I32)
        idxs = []
        for c in range(C):
            kmax = jnp.max(jnp.max(keys, axis=0, keepdims=True), axis=1, keepdims=True)
            keys = jnp.where(keys == kmax, 0.0, keys)
            kbits = pltpu.bitcast(jnp.broadcast_to(kmax, (C, 128)), I32)
            top = jnp.where(crow == c, kbits, top)
            idx = jnp.max((S - 1 - (kbits & (S - 1))).astype(F32)).astype(I32)
            idxs.append(jnp.clip(idx, 0, S - 1))
            sel_buf[pl.ds(c, 1), :] = act_buf[pl.ds(A_XN + idxs[c], 1), :]
        rank = lax.shift_right_logical(top - KEY_BIAS, 11)
        rbits = jnp.where(rank >= 0x8000, rank - 0x8000, 0xFFFF - rank)
        r_sel = pltpu.bitcast(rbits << 16, F32)[:, 0:1]
        xs = pltpu.bitcast(sel_buf[...], F32)
        gate = _rnd(_silu(_rnd(_nt(xs, wg_buf[...]))))
        up = _rnd(_nt(xs, wu_buf[...]))
        y = _rnd(_nn(_rnd(gate * up), wd_buf[...]))
        y = _rnd(y * _rnd(jax.nn.sigmoid(r_sel)))
        g_sel = pltpu.bitcast(_rnd(_silu(_rnd(xs + y))), U32)
        for c in range(C):
            act_buf[pl.ds(A_G + idxs[c], 1), :] = g_sel[c:c + 1]

    def scan(out_buf, sems, pm_buf, *raw):
        o_buf, px_buf, km_buf, vm_buf, om_buf = (r.bitcast(BF) for r in raw)
        o_buf[:, pl.ds(0, FRONT), :] = jnp.zeros((NQ, FRONT, 4 * E), BF)
        row = lax.broadcasted_iota(I32, (M + SEG, NK), 0) - M
        col = lax.broadcasted_iota(I32, (M + SEG, NK), 1)
        visible = ((col <= row) | (row < 0) | (col >= SEG)) & (col < SEG + M)
        fill = jnp.where(col < SEG + M, -1e9 * LOG2E, -jnp.inf).astype(F32)
        zeros = jnp.zeros((M, 4 * E), F32)

        def finish(r, n, s):
            x = x_buf[pl.ds(r, n), :].astype(F32)
            out_buf[pl.ds(r, n), :] = (x + _rnd(_rnd(s) * act(A_G - FRONT, r, n))).astype(BF)

        def step(s, odd, mem, last=None):
            seg = _aligned(s * SEG, SEG)
            rin = _aligned(PRO + RIDE * s, 8)
            rout = _aligned(RIDE * (s - 1) + FRONT, 8)
            win = _aligned(rin - 8 * odd, 16)
            wout = _aligned(rout - 8 * (1 - odd), 16)
            lhs = _cat([mem, act(A_XN, rin, RIDE)]).astype(BF)
            qm, om, acc = {}, {}, []

            def lanes(h):
                return slice(h % 4 * E, (h % 4 + 1) * E)

            def seg_rows(m, h):
                j = h // 4
                return qkv[2 * m + j % 2][j // 2, pl.ds(seg, SEG), lanes(h)]

            def with_mem(m, h):
                return _cat([seg_rows(m, h), (km_buf if m == 1 else vm_buf)[h // 4, :, lanes(h)]])

            def px(h):
                return px_buf.at[h // 4, :, pl.ds(h % 4 * E, NK)]

            def put_o(h, o):
                o_buf.at[h // 4][pl.ds(seg + FRONT, SEG), lanes(h)] = o.astype(BF)

            def project(j, m):
                w = quad_weight(j, m)
                y = _nn(lhs[:, 0:E], w[0:E])
                for k in range(E, D, E):
                    y += _nn(lhs[:, k:k + E], w[k:k + E])
                dst = qkv[2 * m + j % 2].at[j // 2, pl.ds(win, 32), :]
                if odd:
                    dst[8:16, :] = y[8:16].astype(BF)
                    dst[16:32, :] = y[16:32].astype(BF)
                else:
                    dst[0:16, :] = y[8:24].astype(BF)
                    dst[16:24, :] = y[24:32].astype(BF)
                if m == 0:
                    qm[j] = _rnd(y[0:M])
                else:
                    (km_buf if m == 1 else vm_buf).at[j][...] = _cat([y[0:M], zeros]).astype(BF)

            def softmax(q, h):
                r0 = M + SEG - q.shape[0]
                sc = _nt(q, with_mem(1, h)) * (E ** -0.5 * LOG2E)
                sc = jnp.where(visible[r0:], sc, fill[r0:])
                e = jnp.exp2(sc - jnp.max(sc, axis=1, keepdims=True))
                return e * _recip(jnp.sum(e, axis=1, keepdims=True))

            def scores_seg(h):
                px(h)[...] = softmax(seg_rows(0, h), h).astype(BF)

            def scores(h):
                p = softmax(_cat([qm[h // 4][:, lanes(h)], seg_rows(0, h).astype(F32)]), h)
                if h < H - TAIL:
                    pm_buf[h] = _rnd(p)
                else:
                    pm_buf[h, 0:M] = _rnd(p[0:M])
                    px(h)[...] = p[M:].astype(BF)

            def mix(h):
                o = _nn(pm_buf[h], with_mem(2, h))
                om[h] = o[0:M]
                put_o(h, o[M:])

            def mix_mem(h):
                om[h] = _nn(pm_buf[h, 0:M], with_mem(2, h))

            def mix_seg(h):
                put_o(h, _nn(px(h)[...], with_mem(2, h)))

            def out_proj(h):
                lo = o_buf[h // 4, pl.ds(wout, 16), lanes(h)]
                hi = o_buf[h // 4, pl.ds(wout + 16, 16), lanes(h)]
                full, half = (lo, hi.astype(F32)[0:8]) if odd else (hi, lo.astype(F32)[8:16])
                om_buf.at[h // 4][:, lanes(h)] = _cat([om[h], half]).astype(BF)
                y = _nn(_cat([om_buf[h // 4, :, lanes(h)], full]), _as_bf(wo_buf[h]))
                acc[:] = [acc[0] + y if acc else y]

            order = [(3 * j + m, project, j, m) for j in range(NQ) for m in range(3)]
            if last:
                order.append((3 * NQ + 1, last))
                for h in range(H):
                    t = 3 * (h // 4)
                    order += [(t + 3.5, scores_seg, h), (t + 7.5, mix_seg, h)]
                for _, fn, *args in sorted(order, key=lambda e: e[0]):
                    fn(*args)
                return None
            order += [(3 * NQ + h / 4, out_proj, h) for h in range(H)]
            for h in range(H):
                t = 3 * (h // 4)
                order.append((t + 3.5, scores, h))
                if h < H - TAIL:
                    order.append((t + 7.5, mix, h))
                else:
                    order += [(t + 6.4, mix_mem, h), (4 * NQ, mix_seg, h)]
            for _, fn, *args in sorted(order, key=lambda e: e[0]):
                fn(*args)

            y = acc[0]
            finish(rout, RIDE, _cat([y[16:32], y[8:16]]) if odd else y[8:32])
            return _rnd(y[0:M])

        def steps(i, mem, n=UNROLL):
            for k in range(n):
                mem = step(UNROLL * i + k, k % 2, mem)
            return mem

        copies = []

        def write_out(t, n):
            copies.append(pltpu.make_async_copy(out_buf.at[pl.ds(FRONT + t, n)],
                                                out_hbm.at[pl.ds(t, n)], sems.at[len(copies)]))
            copies[-1].start()

        def epilogue(b):
            t, n = EPI0 + sum(EPI_BLOCKS[:b]), EPI_BLOCKS[b]
            o = _cat([o_buf[j, pl.ds(FRONT + t, n), :] for j in range(NQ)], 1)
            finish(FRONT + t, n, _nn(o, _as_bf(wo_buf[...].reshape(H * E // 2, D))))
            return t, n

        nloop = NSEG // UNROLL - 1
        mem = lax.fori_loop(0, nloop, steps, mem_buf[...].astype(F32))
        mem = steps(nloop, mem, UNROLL - 1)
        step(NSEG - 1, 1, mem, functools.partial(epilogue, 0))
        write_out(0, EPI0 + EPI_BLOCKS[0])
        for b in range(1, len(EPI_BLOCKS)):
            write_out(*epilogue(b))
        for cp in copies:
            cp.wait()

    pl.run_scoped(
        prologue,
        pltpu.VMEM((D,), BF),
        *[pltpu.VMEM((FF, D), BF) for _ in range(3)],
        pltpu.VMEM((S // 128, 128), F32),
        pltpu.VMEM((C, D), U32),
        pltpu.SemaphoreType.DMA((9,)),
        pltpu.SemaphoreType.DMA((3 * NQ,)),
    )
    pl.run_scoped(
        scan,
        pltpu.VMEM((FRONT + S, D), BF),
        pltpu.SemaphoreType.DMA((len(EPI_BLOCKS),)),
        pltpu.VMEM((H, M + SEG, NK), F32),
        pltpu.VMEM((NQ, (FRONT + S) // 2, 4 * E), U32),
        pltpu.VMEM((NQ, SEG // 2, 4 * E), U32),
        *[pltpu.VMEM((NQ, 8, 4 * E), U32) for _ in range(3)],
    )


@functools.partial(jax.jit, static_argnames=("A_seg_len",))
def pallas_recurrent_scan__memory_aug_recurrent_mem_tr__moe_arch_mod__prompt_kernel(
    A_x: jax.Array,
    A_mem0: jax.Array,
    A_Wq: jax.Array,
    A_Wk: jax.Array,
    A_Wv: jax.Array,
    A_Wo: jax.Array,
    A_seg_len: int,
    B_x: jax.Array,
    B_w_r: jax.Array,
    B_w_gate: jax.Array,
    B_w_up: jax.Array,
    B_w_down: jax.Array,
):
    del B_x
    assert A_seg_len == SEG and A_x.shape == (1, S, D) and A_mem0.shape == (1, M, D)
    assert A_Wq.shape == (D, H, E) and A_Wo.shape == (H, E, D) and B_w_gate.shape == (D, FF)
    hbm = pl.BlockSpec(memory_space=pltpu.MemorySpace.HBM)
    out = pl.pallas_call(
        _kernel,
        out_shape=jax.ShapeDtypeStruct((S, D), BF),
        in_specs=[hbm] * 10,
        out_specs=hbm,
        scratch_shapes=[
            pltpu.VMEM((FRONT + TOK, D), BF),
            pltpu.VMEM((A_XB + LN0 // 2, D), U32),
            pltpu.VMEM((H, E // 2, D), U32),
            pltpu.VMEM((M, D), BF),
            pltpu.VMEM((3 * H, D // 2, E), U32),
            *[pltpu.VMEM((NQ // 2, QROWS // 2, 4 * E), U32) for _ in range(6)],
        ],
        compiler_params=pltpu.CompilerParams(vmem_limit_bytes=124 * 1024 * 1024),
    )(A_x.reshape(S, D), A_mem0.reshape(M, D),
      *(w.reshape(D // 2, 2, H, E) for w in (A_Wq, A_Wk, A_Wv)), A_Wo,
      B_w_r, B_w_gate.T, B_w_up.T, B_w_down)
    return out.reshape(1, S, D)
```

```python
import functools

import jax
import jax.numpy as jnp
import numpy as np
from jax import lax
import jax.experimental.pallas as pl
import jax.experimental.pallas.tpu as pltpu

BF = jnp.bfloat16
F32 = jnp.float32
U32 = jnp.uint32
I32 = jnp.int32

S, D, H, E, M, SEG, FF, C = 2048, 640, 32, 128, 8, 32, 1728, 8
NSEG = S // SEG
NQ = H // 4
RIDE = 24
PRO_BLOCKS = (144, 128, 128, 128)
PRO = sum(PRO_BLOCKS)
EPI_BLOCKS = (192, 192, 128, 48)
EPI0 = S - sum(EPI_BLOCKS)
FRONT = 32
QROWS = PRO + RIDE * NSEG
LN0 = PRO
LNJ = 256
TOK = LN0 + 6 * LNJ
A_XN, A_G, A_XB = 0, TOK + FRONT, TOK + FRONT + S
NK = SEG + 16
UNROLL = 4
TAIL = 10
KEY_BIAS = 0x10000000
LN_EPS = 1.0013580322265625e-05
LOG2E = 1.4426950408889634


def _nn(a, b):
    return lax.dot_general(a, b, (((1,), (0,)), ((), ())), preferred_element_type=F32)


def _nt(a, b):
    return lax.dot_general(a, b, (((1,), (1,)), ((), ())), preferred_element_type=F32)


def _as_bf(x):
    return pltpu.bitcast(x, BF)


def _rnd(x):
    return x.astype(BF).astype(F32)


def _cat(xs, axis=0):
    return jnp.concatenate(xs, axis)


def _recip(x):
    r = pl.reciprocal(x, approx=True)
    return r * (2.0 - x * r)


def _silu(x):
    return x * jax.nn.sigmoid(x)


def _aligned(x, n):
    return x if isinstance(x, int) else pl.multiple_of(x, n)


def _interleave(*gens):
    gens = list(gens)
    while gens:
        gens = [g for g in gens if next(g, StopIteration) is not StopIteration]


def _kernel(x_hbm, mem_hbm, wq_hbm, wk_hbm, wv_hbm, wo_hbm, wr_hbm, wg_hbm, wu_hbm, wd_hbm,
            out_hbm, x_buf, act_buf, wo_buf, mem_buf, w_buf, *qkv_raw):
    qkv = [r.bitcast(BF) for r in qkv_raw]

    def act(base, r, n):
        return pltpu.bitcast(act_buf[pl.ds(base + r, n), :], F32)

    def set_act(base, r, val):
        act_buf[pl.ds(base + r, val.shape[0]), :] = pltpu.bitcast(val, U32)

    def quad_weight(j, m):
        return _as_bf(_cat([w_buf[4 * (3 * j + m) + t] for t in range(4)], 1))

    def prologue(wr_buf, wg_buf, wu_buf, wd_buf, key_buf, sel_buf, sems, wsems):
        srcs = [w.bitcast(U32) for w in (wq_hbm, wk_hbm, wv_hbm)]
        copy = pltpu.make_async_copy
        cp_x0 = copy(x_hbm.at[pl.ds(0, LN0)], x_buf.at[pl.ds(FRONT, LN0)], sems.at[0])
        cp_x1 = copy(x_hbm.at[pl.ds(LN0, LNJ)], x_buf.at[pl.ds(FRONT + LN0, LNJ)], sems.at[1])
        cp_x2 = copy(x_hbm.at[pl.ds(LN0 + LNJ, S - LN0 - LNJ)],
                     x_buf.at[pl.ds(FRONT + LN0 + LNJ, S - LN0 - LNJ)], sems.at[8])
        cp_wr = copy(wr_hbm, wr_buf, sems.at[2])
        cp_mem = copy(mem_hbm, mem_buf, sems.at[3])
        cp_wo = copy(wo_hbm.bitcast(U32), wo_buf, sems.at[4])
        cp_wg = copy(wg_hbm, wg_buf, sems.at[5])
        cp_wu = copy(wu_hbm, wu_buf, sems.at[6])
        cp_wd = copy(wd_hbm, wd_buf, sems.at[7])

        def weight_copies(i, *units):
            return [copy(srcs[k % 3].at[:, t % 2, 2 * (2 * i + k // 3) + t // 2, :],
                         w_buf.at[4 * (6 * i + k) + t], wsems.at[6 * i + k])
                    for k in units for t in range(4)]

        def start(copies):
            for cp in copies:
                cp.start()

        def wait(copies):
            for cp in copies:
                cp.wait()

        def unzip(u):
            for t in (0, 2):
                for r in (0, D // 4):
                    rows = pl.ds(r, D // 4)
                    a = w_buf[4 * u + t, rows, :]
                    b = w_buf[4 * u + t + 1, rows, :]
                    w_buf[4 * u + t, rows, :] = (a & np.uint32(0xFFFF)) | (b << 16)
                    w_buf[4 * u + t + 1, rows, :] = (a >> 16) | (b & np.uint32(0xFFFF0000))
                    yield

        def layernorm(t0, n):
            x = x_buf[pl.ds(FRONT + t0, n), :].astype(F32)
            mean = jnp.sum(x, axis=1, keepdims=True) / D
            cen = x - mean
            var = jnp.sum(cen * cen, axis=1, keepdims=True) / D
            den = _rnd(jnp.sqrt(_rnd(_rnd(var) + LN_EPS)))
            xn = _rnd(_rnd(x - _rnd(mean)) * (1.0 / den))
            set_act(A_XN, t0, xn)
            return xn

        def layernorm_pieces(t0):
            for p in range(4):
                layernorm(pl.multiple_of(t0 + p * (LNJ // 4), 16), LNJ // 4)
                yield

        def gate_pieces(blk):
            wr = wr_buf[...].astype(F32).reshape(1, D)
            best = None
            for p in range(0, 128, 32):
                t0 = _aligned(blk * 128 + p, 32)
                xn = act(A_XN, t0, 32)
                set_act(A_G, t0, _rnd(xn * _recip(1.0 + jnp.exp(-xn))))
                r = jnp.broadcast_to(_rnd(jnp.sum(xn * wr, axis=1, keepdims=True)), (32, 128))
                bits = lax.shift_right_logical(pltpu.bitcast(r, I32), 16)
                rank = jnp.where(r < 0, 0xFFFF - bits, (bits & 0x7FFF) + 0x8000)
                rank = jnp.where(r != r, 0, rank)
                row = lax.broadcasted_iota(I32, (32, 128), 0) + p
                lane = lax.broadcasted_iota(I32, (32, 128), 1)
                key = KEY_BIAS + rank * S + (S - 1 - blk * 128 - lane)
                key = pltpu.bitcast(jnp.where(row == lane, key, 0), F32)
                best = key if best is None else jnp.maximum(best, key)
                yield
            key_buf[pl.ds(blk, 1), :] = jnp.max(best, axis=0, keepdims=True)

        def project_pieces(i, k):
            j, m, odd = 2 * i + k // 3, k % 3, k // 3 % 2
            r = 0
            for n in PRO_BLOCKS:
                y = _nn(_as_bf(act_buf[pl.ds(A_XB + r // 2, n // 2), :]), quad_weight(j, m))
                qkv[2 * m + odd].at[j // 2][pl.ds(r, n), :] = y.astype(BF)
                r += n
                yield

        start([cp_x0, cp_wr, *weight_copies(0, 0)])
        x_buf[pl.ds(0, FRONT), :] = jnp.zeros((FRONT, D), BF)
        x_buf[pl.ds(FRONT + S, TOK - S), :] = jnp.zeros((TOK - S, D), BF)
        set_act(A_G - FRONT, 0, jnp.zeros((FRONT, D), F32))
        wait([cp_x0, cp_wr])
        start(weight_copies(0, 1))

        def first_layernorm(i, carry):
            n = LN0 // 3
            xn = layernorm(pl.multiple_of(i * n, 16), n)
            act_buf[pl.ds(pl.multiple_of(A_XB + i * (n // 2), 8), n // 2), :] = pltpu.bitcast(
                xn.astype(BF), U32)
            pl.when(i == 0)(lambda: start([*weight_copies(0, 2, 3, 4), cp_x1]))
            return i - 1

        one = lax.fori_loop(0, 3, first_layernorm, 0)
        wait(weight_copies(0, 0, 1))
        _interleave(unzip(0))
        _interleave(project_pieces(0, 0), unzip(1), gate_pieces(one - 1), gate_pieces(one))

        def six_units(i, carry):
            for half in range(2):
                k0 = 3 * half + 1
                wait(weight_copies(i, k0 + 1, k0 + 2, k0 + 3))
                pl.when(i == 0)((cp_x2 if half else cp_x1).wait)
                start(weight_copies(i, k0 + 4, k0 + 5, k0 + 6))
                for k, cp in enumerate((cp_wo, cp_wu, cp_mem) if half else (cp_x2, cp_wg, cp_wd)):
                    pl.when(i == k)(cp.start)
                blk = 4 * i + 2 * half + 2
                sides = (gate_pieces(blk), gate_pieces(blk + 1),
                         layernorm_pieces(LN0 + (2 * i + half) * LNJ))
                for k, side in zip(range(k0, k0 + 3), sides):
                    _interleave(project_pieces(i, k), unzip(6 * i + k + 1), side)
            return blk + 2

        blk = lax.fori_loop(0, 3, six_units, 0)
        start(weight_copies(3, 5))
        wait(weight_copies(3, 2, 3, 4))
        _interleave(project_pieces(3, 1), unzip(20), gate_pieces(blk), gate_pieces(blk + 1))
        wait([*weight_copies(3, 5), cp_wg, cp_wu, cp_wd, cp_wo, cp_mem])
        _interleave(project_pieces(3, 2), unzip(21), unzip(22), unzip(23))

        keys = key_buf[...]
        crow = lax.broadcasted_iota(I32, (C, 128), 0)
        top = jnp.zeros((C, 128), I32)
        idxs = []
        for c in range(C):
            kmax = jnp.max(jnp.max(keys, axis=0, keepdims=True), axis=1, keepdims=True)
            keys = jnp.where(keys == kmax, 0.0, keys)
            kbits = pltpu.bitcast(jnp.broadcast_to(kmax, (C, 128)), I32)
            top = jnp.where(crow == c, kbits, top)
            idx = jnp.max((S - 1 - (kbits & (S - 1))).astype(F32)).astype(I32)
            idxs.append(jnp.clip(idx, 0, S - 1))
            sel_buf[pl.ds(c, 1), :] = act_buf[pl.ds(A_XN + idxs[c], 1), :]
        rank = lax.shift_right_logical(top - KEY_BIAS, 11)
        rbits = jnp.where(rank >= 0x8000, rank - 0x8000, 0xFFFF - rank)
        r_sel = pltpu.bitcast(rbits << 16, F32)[:, 0:1]
        xs = pltpu.bitcast(sel_buf[...], F32)

        def project_with(k, small):
            j, m, odd = 6 + k // 3, k % 3, k // 3 % 2
            w = quad_weight(j, m)
            r = 0
            for n in PRO_BLOCKS:
                x = _as_bf(act_buf[pl.ds(A_XB + r // 2, n // 2), :])
                y = None
                for c in range(0, D, E):
                    yc = _nn(x[:, c:c + E], w[c:c + E])
                    y = yc if y is None else y + yc
                    next(small, None)
                qkv[2 * m + odd].at[j // 2][pl.ds(r, n), :] = y.astype(BF)
                r += n
            _interleave(small)

        def ffn_in(w_ref, out):
            for f in range(0, FF, 4 * E):
                z = None
                for c in range(0, D, E):
                    zc = _nt(xs[:, c:c + E], w_ref[f:min(f + 4 * E, FF), c:c + E])
                    z = zc if z is None else z + zc
                    yield
                out.append(z)

        def ffn_out(hid, out):
            for f in range(0, FF, E):
                zc = _nn(hid[:, f:min(f + E, FF)], wd_buf[f:min(f + E, FF), :])
                out[:] = [out[0] + zc if out else zc]
                yield

        gate, up, down = [], [], []
        project_with(3, ffn_in(wg_buf, gate))
        project_with(4, ffn_in(wu_buf, up))
        hid = _rnd(_rnd(_silu(_rnd(_cat(gate, 1)))) * _rnd(_cat(up, 1)))
        project_with(5, ffn_out(hid, down))
        y = _rnd(down[0])
        y = _rnd(y * _rnd(jax.nn.sigmoid(r_sel)))
        g_sel = pltpu.bitcast(_rnd(_silu(_rnd(xs + y))), U32)
        for c in range(C):
            act_buf[pl.ds(A_G + idxs[c], 1), :] = g_sel[c:c + 1]

    def scan(out_buf, sems, pm_buf, *raw):
        o_buf, px_buf, km_buf, vm_buf, om_buf = (r.bitcast(BF) for r in raw)
        o_buf[:, pl.ds(0, FRONT), :] = jnp.zeros((NQ, FRONT, 4 * E), BF)
        row = lax.broadcasted_iota(I32, (M + SEG, NK), 0) - M
        col = lax.broadcasted_iota(I32, (M + SEG, NK), 1)
        visible = ((col <= row) | (row < 0) | (col >= SEG)) & (col < SEG + M)
        fill = jnp.where(col < SEG + M, -1e9 * LOG2E, -jnp.inf).astype(F32)
        zeros = jnp.zeros((M, 4 * E), F32)

        def finish(r, n, s):
            x = x_buf[pl.ds(r, n), :].astype(F32)
            out_buf[pl.ds(r, n), :] = (x + _rnd(_rnd(s) * act(A_G - FRONT, r, n))).astype(BF)

        def step(s, odd, mem, last=None):
            seg = _aligned(s * SEG, SEG)
            rin = _aligned(PRO + RIDE * s, 8)
            rout = _aligned(RIDE * (s - 1) + FRONT, 8)
            win = _aligned(rin - 8 * odd, 16)
            wout = _aligned(rout - 8 * (1 - odd), 16)
            lhs = _cat([mem, act(A_XN, rin, RIDE)]).astype(BF)
            qm, om, acc = {}, {}, []

            def lanes(h):
                return slice(h % 4 * E, (h % 4 + 1) * E)

            def seg_rows(m, h):
                j = h // 4
                return qkv[2 * m + j % 2][j // 2, pl.ds(seg, SEG), lanes(h)]

            def with_mem(m, h):
                return _cat([seg_rows(m, h), (km_buf if m == 1 else vm_buf)[h // 4, :, lanes(h)]])

            def px(h):
                return px_buf.at[h // 4, :, pl.ds(h % 4 * E, NK)]

            def put_o(h, o):
                o_buf.at[h // 4][pl.ds(seg + FRONT, SEG), lanes(h)] = o.astype(BF)

            def project(j, m):
                w = quad_weight(j, m)
                y = _nn(lhs[:, 0:E], w[0:E])
                for k in range(E, D, E):
                    y += _nn(lhs[:, k:k + E], w[k:k + E])
                dst = qkv[2 * m + j % 2].at[j // 2, pl.ds(win, 32), :]
                if odd:
                    dst[8:16, :] = y[8:16].astype(BF)
                    dst[16:32, :] = y[16:32].astype(BF)
                else:
                    dst[0:16, :] = y[8:24].astype(BF)
                    dst[16:24, :] = y[24:32].astype(BF)
                if m == 0:
                    qm[j] = _rnd(y[0:M])
                else:
                    (km_buf if m == 1 else vm_buf).at[j][...] = _cat([y[0:M], zeros]).astype(BF)

            def softmax(q, h):
                r0 = M + SEG - q.shape[0]
                sc = _nt(q, with_mem(1, h)) * (E ** -0.5 * LOG2E)
                sc = jnp.where(visible[r0:], sc, fill[r0:])
                e = jnp.exp2(sc - jnp.max(sc, axis=1, keepdims=True))
                return e * _recip(jnp.sum(e, axis=1, keepdims=True))

            def scores_seg(h):
                px(h)[...] = softmax(seg_rows(0, h), h).astype(BF)

            def scores(h):
                p = softmax(_cat([qm[h // 4][:, lanes(h)], seg_rows(0, h).astype(F32)]), h)
                if h < H - TAIL:
                    pm_buf[h] = _rnd(p)
                else:
                    pm_buf[h, 0:M] = _rnd(p[0:M])
                    px(h)[...] = p[M:].astype(BF)

            def mix(h):
                o = _nn(pm_buf[h], with_mem(2, h))
                om[h] = o[0:M]
                put_o(h, o[M:])

            def mix_mem(h):
                om[h] = _nn(pm_buf[h, 0:M], with_mem(2, h))

            def mix_seg(h):
                put_o(h, _nn(px(h)[...], with_mem(2, h)))

            def out_proj(h):
                lo = o_buf[h // 4, pl.ds(wout, 16), lanes(h)]
                hi = o_buf[h // 4, pl.ds(wout + 16, 16), lanes(h)]
                full, half = (lo, hi.astype(F32)[0:8]) if odd else (hi, lo.astype(F32)[8:16])
                om_buf.at[h // 4][:, lanes(h)] = _cat([om[h], half]).astype(BF)
                y = _nn(_cat([om_buf[h // 4, :, lanes(h)], full]), _as_bf(wo_buf[h]))
                acc[:] = [acc[0] + y if acc else y]

            order = [(3 * j + m, project, j, m) for j in range(NQ) for m in range(3)]
            if last:
                order.append((3 * NQ + 1, last))
                for h in range(H):
                    t = 3 * (h // 4)
                    order += [(t + 3.5, scores_seg, h), (t + 7.5, mix_seg, h)]
                for _, fn, *args in sorted(order, key=lambda e: e[0]):
                    fn(*args)
                return None
            order += [(3 * NQ + h / 4, out_proj, h) for h in range(H)]
            for h in range(H):
                t = 3 * (h // 4)
                order.append((t + 3.5, scores, h))
                if h < H - TAIL:
                    order.append((t + 7.5, mix, h))
                else:
                    order += [(t + 6.4, mix_mem, h), (4 * NQ, mix_seg, h)]
            for _, fn, *args in sorted(order, key=lambda e: e[0]):
                fn(*args)

            y = acc[0]
            finish(rout, RIDE, _cat([y[16:32], y[8:16]]) if odd else y[8:32])
            return _rnd(y[0:M])

        def steps(i, mem, n=UNROLL):
            for k in range(n):
                mem = step(UNROLL * i + k, k % 2, mem)
            return mem

        copies = []

        def write_out(t, n):
            copies.append(pltpu.make_async_copy(out_buf.at[pl.ds(FRONT + t, n)],
                                                out_hbm.at[pl.ds(t, n)], sems.at[len(copies)]))
            copies[-1].start()

        def epilogue(b):
            t, n = EPI0 + sum(EPI_BLOCKS[:b]), EPI_BLOCKS[b]
            o = _cat([o_buf[j, pl.ds(FRONT + t, n), :] for j in range(NQ)], 1)
            finish(FRONT + t, n, _nn(o, _as_bf(wo_buf[...].reshape(H * E // 2, D))))
            return t, n

        nloop = (NSEG - 1) // UNROLL
        mem = lax.fori_loop(0, nloop, steps, mem_buf[...].astype(F32))
        mem = steps(nloop, mem, NSEG - 1 - nloop * UNROLL)
        step(NSEG - 1, 1, mem, functools.partial(epilogue, 0))
        write_out(0, EPI0 + EPI_BLOCKS[0])
        for b in range(1, len(EPI_BLOCKS)):
            write_out(*epilogue(b))
        for cp in copies:
            cp.wait()

    pl.run_scoped(
        prologue,
        pltpu.VMEM((D,), BF),
        *[pltpu.VMEM((FF, D), BF) for _ in range(3)],
        pltpu.VMEM((S // 128, 128), F32),
        pltpu.VMEM((C, D), U32),
        pltpu.SemaphoreType.DMA((9,)),
        pltpu.SemaphoreType.DMA((3 * NQ,)),
    )
    pl.run_scoped(
        scan,
        pltpu.VMEM((FRONT + S, D), BF),
        pltpu.SemaphoreType.DMA((len(EPI_BLOCKS),)),
        pltpu.VMEM((H, M + SEG, NK), F32),
        pltpu.VMEM((NQ, (FRONT + S) // 2, 4 * E), U32),
        pltpu.VMEM((NQ, SEG // 2, 4 * E), U32),
        *[pltpu.VMEM((NQ, 8, 4 * E), U32) for _ in range(3)],
    )


@functools.partial(jax.jit, static_argnames=("A_seg_len",))
def pallas_recurrent_scan__memory_aug_recurrent_mem_tr__moe_arch_mod__prompt_kernel(
    A_x: jax.Array,
    A_mem0: jax.Array,
    A_Wq: jax.Array,
    A_Wk: jax.Array,
    A_Wv: jax.Array,
    A_Wo: jax.Array,
    A_seg_len: int,
    B_x: jax.Array,
    B_w_r: jax.Array,
    B_w_gate: jax.Array,
    B_w_up: jax.Array,
    B_w_down: jax.Array,
):
    del B_x
    assert A_seg_len == SEG and A_x.shape == (1, S, D) and A_mem0.shape == (1, M, D)
    assert A_Wq.shape == (D, H, E) and A_Wo.shape == (H, E, D) and B_w_gate.shape == (D, FF)
    hbm = pl.BlockSpec(memory_space=pltpu.MemorySpace.HBM)
    out = pl.pallas_call(
        _kernel,
        out_shape=jax.ShapeDtypeStruct((S, D), BF),
        in_specs=[hbm] * 10,
        out_specs=hbm,
        scratch_shapes=[
            pltpu.VMEM((FRONT + TOK, D), BF),
            pltpu.VMEM((A_XB + LN0 // 2, D), U32),
            pltpu.VMEM((H, E // 2, D), U32),
            pltpu.VMEM((M, D), BF),
            pltpu.VMEM((3 * H, D // 2, E), U32),
            *[pltpu.VMEM((NQ // 2, QROWS // 2, 4 * E), U32) for _ in range(6)],
        ],
        compiler_params=pltpu.CompilerParams(vmem_limit_bytes=124 * 1024 * 1024),
    )(A_x.reshape(S, D), A_mem0.reshape(M, D),
      *(w.reshape(D // 2, 2, H, E) for w in (A_Wq, A_Wk, A_Wv)), A_Wo,
      B_w_r, B_w_gate.T, B_w_up.T, B_w_down)
    return out.reshape(1, S, D)
```
